```python
import jax
import jax.numpy as jnp

def _softmax(x, axis=-1):
    return jax.nn.softmax(x, axis=axis)

def _gelu(x):
    return jax.nn.gelu(x, approximate=True)

def _silu(x):
    return jax.nn.silu(x)

def _sigmoid(x):
    return jax.nn.sigmoid(x)

def _layernorm(x, axis=-1, eps=1e-05):
    m = jnp.mean(x, axis=axis, keepdims=True)
    v = jnp.var(x, axis=axis, keepdims=True)
    return (x - m) / jnp.sqrt(v + eps)

def _scatter_add(tgt, idx, src, axis=0):
    return tgt.at[idx].add(src)

def _segment_sum(src, seg, n):
    return jax.ops.segment_sum(src, seg, n)

class _Rng:

    def __init__(self, key):
        self._k = key

    def _next(self):
        self._k, sub = jax.random.split(self._k)
        return sub

    def normal(self, shape):
        return jax.random.normal(self._next(), shape, dtype=jnp.bfloat16)

    def randint(self, lo, hi, shape):
        return jax.random.randint(self._next(), shape, lo, hi, dtype=jnp.int32)

    def uniform(self, shape, lo=0.0, hi=1.0):
        return jax.random.uniform(self._next(), shape, jnp.bfloat16, lo, hi)

    def permutation(self, n):
        return jax.random.permutation(self._next(), n)
kernel_name = 'gated_mix__memory_aug_recurrent_mem_tr__ssm_conv_h3__prompt'

def setup_inputs():
    _rng = _Rng(jax.random.key(int.from_bytes(__import__("os").urandom(4), "little")))
    _w = lambda a: (lambda t: t.astype(jnp.bfloat16) if jnp.issubdtype(t.dtype, jnp.floating) else t)(jnp.asarray(a))

    def _A_setup():
        B, S, Dm = (1, 2048, 640)
        H, Dh = (32, 192)
        M, seg = (8, 32)
        seg = min(seg, S)
        S = S // seg * seg
        return {'x': _w((lambda *s: _rng.normal(s) * 0.05)(B, S, Dm)), 'mem0': _w((lambda *s: _rng.normal(s) * 0.05)(B, M, Dm)), 'Wq': _w((lambda *s: _rng.normal(s) * 0.05)(Dm, H, Dh) * Dm ** (-0.5)), 'Wk': _w((lambda *s: _rng.normal(s) * 0.05)(Dm, H, Dh) * Dm ** (-0.5)), 'Wv': _w((lambda *s: _rng.normal(s) * 0.05)(Dm, H, Dh) * Dm ** (-0.5)), 'Wo': _w((lambda *s: _rng.normal(s) * 0.05)(H, Dh, Dm) * (H * Dh) ** (-0.5)), 'seg_len': seg}
    _A_in = _A_setup()

    def _B_setup():
        B, S, D = (1, 2048, 640)
        ks = 4
        return {'q': _w((lambda *s: _rng.normal(s) * 0.05)(B, S, D)), 'k': _w((lambda *s: _rng.normal(s) * 0.05)(B, S, D)), 'v': _w((lambda *s: _rng.normal(s) * 0.05)(B, S, D)), 'shift_k': _w((lambda *s: _rng.normal(s) * 0.05)(D, ks) * 0.5), 'ssm_k': _w((lambda *s: _rng.normal(s) * 0.05)(D, S) * (1.0 / S ** 0.5)), 'ssm_D': _w((lambda *s: _rng.normal(s) * 0.05)(D))}
    _B_in = _B_setup()
    return {'A_x': _A_in['x'], 'A_mem0': _A_in['mem0'], 'A_Wq': _A_in['Wq'], 'A_Wk': _A_in['Wk'], 'A_Wv': _A_in['Wv'], 'A_Wo': _A_in['Wo'], 'A_seg_len': _A_in['seg_len'], 'B_q': _B_in['q'], 'B_k': _B_in['k'], 'B_v': _B_in['v'], 'B_shift_k': _B_in['shift_k'], 'B_ssm_k': _B_in['ssm_k'], 'B_ssm_D': _B_in['ssm_D'], 'gate_w': _w((lambda *s: _rng.normal(s) * 0.05)(640))}

def reference(A_x, A_mem0, A_Wq, A_Wk, A_Wv, A_Wo, A_seg_len, B_q, B_k, B_v, B_shift_k, B_ssm_k, B_ssm_D, gate_w):

    def _A_ref(x, mem0, Wq, Wk, Wv, Wo, seg_len):
        B, S, Dm = x.shape
        H, Dh = (Wq.shape[1], Wq.shape[2])
        M = mem0.shape[1]
        scale = Dh ** (-0.5)
        n_seg = S // seg_len
        L = M + seg_len
        idx = jnp.arange(L)
        mask = (idx[:, None] < M) | (idx[:, None] >= idx[None, :])
        mem = mem0
        outs = []
        for s in range(n_seg):
            xs = x[:, s * seg_len:(s + 1) * seg_len, :].copy()
            h = jnp.concatenate([mem, xs], axis=1)
            q = jnp.einsum('btd,dhe->bhte', h, Wq)
            k = jnp.einsum('btd,dhe->bhte', h, Wk)
            v = jnp.einsum('btd,dhe->bhte', h, Wv)
            scores = jnp.einsum('bhqe,bhke->bhqk', q, k) * scale
            scores = jnp.where(mask[None, None], scores, -1000000000.0)
            p = _softmax(scores, axis=-1)
            o = jnp.einsum('bhqk,bhke->bhqe', p, v)
            o = jnp.einsum('bhte,hed->btd', o, Wo)
            mem = o[:, :M, :].copy()
            outs.append(o[:, M:, :])
        return jnp.concatenate(outs, axis=1)

    def _B_ref(q, k, v, shift_k, ssm_k, ssm_D):
        B, S, D = q.shape
        ks = shift_k.shape[-1]
        k_pad = jnp.pad(k, ((0, 0), (ks - 1, 0), (0, 0)))
        k_shift = jnp.zeros_like(k)
        for t in range(ks):
            k_shift = k_shift + k_pad[:, t:t + S, :] * shift_k[:, ks - 1 - t][None, None, :]
        kv = k_shift * v
        L = 2 * S
        kv_pad = jnp.pad(kv, ((0, 0), (0, S), (0, 0)))
        kf_pad = jnp.pad(ssm_k, ((0, 0), (0, S)))
        kv_f = (lambda x, axes=(-2, -1): jnp.fft.rfft2(x.astype(jnp.float32), axes=axes))(kv_pad[:, None, :, :], axes=(1, 2))
        kf_f = (lambda x, axes=(-2, -1): jnp.fft.rfft2(x.astype(jnp.float32), axes=axes))(kf_pad[:, None, :], axes=(1, 2))
        kf_f = (lambda x, *d: x.transpose(*d))(kf_f, 1, 2, 0)
        y_f = kv_f * kf_f[None, :, :, :]
        y = (lambda x, s, axes=(-2, -1): jnp.fft.irfft2(x, s=s, axes=axes).astype(jnp.bfloat16))(y_f, (1, L), axes=(1, 2))[:, 0, :S, :]
        y = y + kv * ssm_D[None, None, :]
        return q * y
    x = A_x
    g = _sigmoid((x * gate_w).sum(-1, keepdims=True))
    a = _A_ref(x, A_mem0, A_Wq, A_Wk, A_Wv, A_Wo, A_seg_len)
    b = _B_ref(x, B_k, B_v, B_shift_k, B_ssm_k, B_ssm_D)
    return g * a + (1 - g) * b
```

```python
import numpy as np

import jax
import jax.numpy as jnp
import jax.experimental.pallas as pl
import jax.experimental.pallas.tpu as pltpu

F32 = jnp.float32
BF16 = jnp.bfloat16
_NN = (((1,), (0,)), ((), ()))
_NT = (((1,), (1,)), ((), ()))
_T = 128


def _dot(a, b, dims=_NN):
    return jax.lax.dot_general(a, b, dims, preferred_element_type=F32)


def _dft_matrices():
    f = np.arange(_T, dtype=np.float64)[:, None]
    n = np.arange(_T, dtype=np.float64)[None, :]
    theta = np.pi * (2.0 * f + 1.0) * n / (2.0 * _T)
    fwd = np.concatenate([np.cos(theta), -np.sin(theta)], axis=0)
    inv = np.concatenate([np.cos(theta).T, -np.sin(theta).T], axis=1) / _T
    return fwd.astype(np.float32), inv.astype(np.float32)


@jax.jit(static_argnames=("A_seg_len",))
def pallas_gated_mix__memory_aug_recurrent_mem_tr__ssm_conv_h3__prompt_kernel(
    A_x: jax.Array,
    A_mem0: jax.Array,
    A_Wq: jax.Array,
    A_Wk: jax.Array,
    A_Wv: jax.Array,
    A_Wo: jax.Array,
    A_seg_len: int,
    B_q: jax.Array,
    B_k: jax.Array,
    B_v: jax.Array,
    B_shift_k: jax.Array,
    B_ssm_k: jax.Array,
    B_ssm_D: jax.Array,
    gate_w: jax.Array,
):
    del B_q
    _, S, D = A_x.shape
    _, H, DH = A_Wq.shape
    M = A_mem0.shape[1]
    SEG = int(A_seg_len)
    KS = B_shift_k.shape[1]
    L = M + SEG
    NSEG = S // SEG
    NP = H // 2
    PW = 2 * DH
    KR = -(-L // 16) * 16
    NB = S // _T
    scale = DH ** -0.5
    assert A_x.shape[0] == 1 and S % SEG == 0 and S % _T == 0 and H % 2 == 0
    assert PW % 128 == 0 and D % 128 == 0 and M % 8 == 0 and SEG % 16 == 0
    assert 2 * KR <= 128 and KS <= 8

    def kernel(x_hbm, mem0_ref, wq_hbm, wk_hbm, wv_hbm, wo_hbm, bk_hbm, bv_hbm,
               shift_ref, ssmk_hbm, ssmd_ref, gw_ref, fwd_ref, inv_ref,
               o_hbm,
               x_v, wqkv, wo_v, h_v, bpart, gate, out_v, in_sems, out_sem):

        def prologue(stage, bk_v, bv_v, ssmk_v, kpad, xf, kf):
            c_ssmk = pltpu.make_async_copy(ssmk_hbm, ssmk_v, in_sems.at[0])
            c_bk = pltpu.make_async_copy(bk_hbm, bk_v, in_sems.at[1])
            c_bv = pltpu.make_async_copy(bv_hbm, bv_v, in_sems.at[2])
            c_x = pltpu.make_async_copy(x_hbm, x_v, in_sems.at[3])
            c_w = [pltpu.make_async_copy(w, stage.at[i], in_sems.at[4 + i])
                   for i, w in enumerate((wq_hbm, wk_hbm, wv_hbm))]
            c_wo = pltpu.make_async_copy(wo_hbm, wo_v, in_sems.at[7])
            for c in (c_ssmk, c_bk, c_bv, c_x, *c_w, c_wo):
                c.start()

            fwd = fwd_ref[...].astype(BF16)
            inv = inv_ref[...].astype(BF16)

            c_ssmk.wait()
            for d in range(NB):
                kf[d] = _dot(fwd, ssmk_v[:, d * _T:(d + 1) * _T], _NT)

            c_bk.wait()
            c_bv.wait()
            taps = shift_ref[...].astype(F32)
            kpad[0:8, :] = jnp.zeros((8, D), F32)

            def fwd_block(a, carry):
                r0 = pl.multiple_of(a * _T, _T)
                kpad[8:8 + _T, :] = bk_v[pl.ds(r0, _T), :].astype(F32)
                ksh = kpad[8:8 + _T, :] * taps[0:1]
                for j in range(1, KS):
                    ksh = ksh + kpad[8 - j:8 - j + _T, :] * taps[j:j + 1]
                kpad[0:8, :] = kpad[_T:_T + 8, :]
                kv = ksh * bv_v[pl.ds(r0, _T), :].astype(F32)
                bpart[pl.ds(r0, _T), :] = kv
                xf[a] = _dot(fwd, kv.astype(BF16))
                return carry

            jax.lax.fori_loop(0, NB, fwd_block, 0)

            sub = jax.lax.broadcasted_iota(jnp.int32, (8, 128), 0)
            sign = (1 - 2 * (sub & 1)).astype(F32)

            def mac(g, carry):
                re = pl.ds(pl.multiple_of(g * 8, 8), 8)
                im = pl.ds(pl.multiple_of(_T + g * 8, 8), 8)
                for t in range(D // 128):
                    ln = slice(t * 128, (t + 1) * 128)
                    xr = [xf[a, re, ln] for a in range(NB)]
                    xi = [xf[a, im, ln] for a in range(NB)]
                    kr = [kf[a, re, ln] for a in range(NB)]
                    ki = [kf[a, im, ln] for a in range(NB)]
                    pr = pi = None
                    for c in range(NB):
                        zr = zi = None
                        for a in range(c + 1):
                            tr = xr[a] * kr[c - a] - xi[a] * ki[c - a]
                            ti = xr[a] * ki[c - a] + xi[a] * kr[c - a]
                            zr = tr if zr is None else zr + tr
                            zi = ti if zi is None else zi + ti
                        if c == 0:
                            wr, wi = zr, zi
                        else:
                            wr, wi = zr - sign * pi, zi + sign * pr
                        pr, pi = zr, zi
                        xf[c, re, ln] = wr
                        xf[c, im, ln] = wi
                return carry

            jax.lax.fori_loop(0, _T // 8, mac, 0)

            c_x.wait()
            skip = ssmd_ref[...].astype(F32).reshape(1, D)
            gw = gw_ref[...].astype(F32).reshape(1, D)

            def inv_block(c, carry):
                rows = pl.ds(pl.multiple_of(c * _T, _T), _T)
                y = _dot(inv, xf[c].astype(BF16))
                xq = x_v[rows, :].astype(F32)
                g = jax.nn.sigmoid(jnp.sum(xq * gw, axis=1, keepdims=True))
                bpart[rows, :] = (1.0 - g) * (xq * (y + bpart[rows, :] * skip))
                gate[rows, :] = jnp.broadcast_to(g, (_T, 128))
                return carry

            jax.lax.fori_loop(0, NB, inv_block, 0)

            for i in range(3):
                c_w[i].wait()

                def transpose(p, carry, i=i):
                    rows = pl.ds(pl.multiple_of(p * PW, PW), PW)
                    wqkv[p, i] = stage[i, rows, :].T
                    return carry

                jax.lax.fori_loop(0, NP, transpose, 0)
            c_wo.wait()

        pl.run_scoped(
            prologue,
            pltpu.VMEM((3, H * DH, D), BF16),
            pltpu.VMEM((S, D), BF16),
            pltpu.VMEM((S, D), BF16),
            pltpu.VMEM((D, S), BF16),
            pltpu.VMEM((_T + 8, D), F32),
            pltpu.VMEM((NB, 2 * _T, D), F32),
            pltpu.VMEM((NB, 2 * _T, D), F32),
        )

        h_v[0:M, :] = mem0_ref[...].astype(F32)

        row = jax.lax.broadcasted_iota(jnp.int32, (L, 2 * KR), 0)
        lane = jax.lax.broadcasted_iota(jnp.int32, (L, 2 * KR), 1)
        in_a = lane < KR
        col = jnp.where(in_a, lane, lane - KR)
        valid = col < L
        valid_a = valid & in_a
        valid_b = valid & (lane >= KR)
        allowed = (row < M) | (row >= col)
        dim_a = jax.lax.broadcasted_iota(jnp.int32, (L, PW), 1) < DH
        zpad = jnp.zeros((KR - L, PW), F32)

        def block_diag(t):
            a = jnp.where(dim_a, t, 0.0)
            b = jnp.where(dim_a, 0.0, t)
            return jnp.concatenate([a, zpad, b, zpad], axis=0).astype(BF16)

        def softmax(s):
            s = jnp.where(allowed, s * scale, -1e9)
            ma = jnp.max(jnp.where(valid_a, s, -jnp.inf), axis=1, keepdims=True)
            mb = jnp.max(jnp.where(valid_b, s, -jnp.inf), axis=1, keepdims=True)
            e = jnp.where(valid, jnp.exp(s - jnp.where(in_a, ma, mb)), 0.0)
            la = jnp.sum(jnp.where(in_a, e, 0.0), axis=1, keepdims=True)
            lb = jnp.sum(jnp.where(in_a, 0.0, e), axis=1, keepdims=True)
            return e * (1.0 / jnp.where(in_a, la, lb))

        def out_copy(s):
            rows = pl.ds(pl.multiple_of(s * SEG, SEG), SEG)
            return pltpu.make_async_copy(out_v.at[rows], o_hbm.at[rows], out_sem)

        def step(s, carry):
            rows = pl.ds(pl.multiple_of(s * SEG, SEG), SEG)
            h_v[M:L, :] = x_v[rows, :].astype(F32)
            h = h_v[...]
            q, k, v, p, o = {}, {}, {}, {}, {}
            acc = []

            def proj_q(i):
                q[i] = _dot(h, wqkv[i, 0])

            def proj_k(i):
                k[i] = block_diag(_dot(h, wqkv[i, 1]))

            def proj_v(i):
                v[i] = block_diag(_dot(h, wqkv[i, 2]))

            def scores(i):
                p[i] = softmax(_dot(q.pop(i), k.pop(i), _NT))

            def values(i):
                o[i] = _dot(p.pop(i), v.pop(i))

            def proj_o(i):
                y = _dot(o.pop(i), wo_v[i * PW:(i + 1) * PW, :])
                acc[:] = [y if not acc else acc[0] + y]

            proj_k(0)
            proj_q(0)
            proj_v(0)
            scores(0)
            for i in range(NP - 1):
                proj_k(i + 1)
                proj_q(i + 1)
                values(i)
                proj_v(i + 1)
                scores(i + 1)
                if i < NP - 3:
                    proj_o(i)
            proj_o(NP - 3)
            values(NP - 1)
            proj_o(NP - 2)
            proj_o(NP - 1)

            y = acc[0]
            h_v[0:M, :] = y[0:M].astype(BF16).astype(F32)
            g = gate[rows, :]
            g = jnp.concatenate([g] * (D // 128), axis=1)
            out_v[rows, :] = (g * y[M:L] + bpart[rows, :]).astype(out_v.dtype)
            out_copy(s).start()
            return carry

        jax.lax.fori_loop(0, NSEG, step, 0)
        pltpu.make_async_copy(out_v, o_hbm, out_sem).wait()

    fwd_np, inv_np = _dft_matrices()
    hbm = pl.BlockSpec(memory_space=pl.ANY)
    vmem = pl.BlockSpec(memory_space=pltpu.VMEM)

    def head_major(w):
        return jnp.transpose(w, (1, 2, 0)).reshape(H * DH, D)

    out = pl.pallas_call(
        kernel,
        out_shape=jax.ShapeDtypeStruct((S, D), A_x.dtype),
        in_specs=[hbm, vmem, hbm, hbm, hbm, hbm, hbm, hbm,
                  vmem, hbm, vmem, vmem, vmem, vmem],
        out_specs=hbm,
        scratch_shapes=[
            pltpu.VMEM((S, D), BF16),
            pltpu.VMEM((NP, 3, D, PW), BF16),
            pltpu.VMEM((H * DH, D), BF16),
            pltpu.VMEM((L, D), F32),
            pltpu.VMEM((S, D), F32),
            pltpu.VMEM((S, 128), F32),
            pltpu.VMEM((S, D), A_x.dtype),
            pltpu.SemaphoreType.DMA((8,)),
            pltpu.SemaphoreType.DMA(()),
        ],
        compiler_params=pltpu.CompilerParams(vmem_limit_bytes=120 * 1024 * 1024),
    )(
        A_x.reshape(S, D), A_mem0.reshape(M, D),
        head_major(A_Wq), head_major(A_Wk), head_major(A_Wv), A_Wo.reshape(H * DH, D),
        B_k.reshape(S, D), B_v.reshape(S, D),
        B_shift_k.T, B_ssm_k, B_ssm_D, gate_w,
        jnp.asarray(fwd_np), jnp.asarray(inv_np),
    )
    return out.reshape(1, S, D)
```

```python
import numpy as np

import jax
import jax.numpy as jnp
import jax.experimental.pallas as pl
import jax.experimental.pallas.tpu as pltpu

F32 = jnp.float32
BF16 = jnp.bfloat16
_NN = (((1,), (0,)), ((), ()))
_NT = (((1,), (1,)), ((), ()))
_T = 128


def _dot(a, b, dims=_NN):
    return jax.lax.dot_general(a, b, dims, preferred_element_type=F32)


def _dft_matrices():
    f = np.arange(_T, dtype=np.float64)[:, None]
    n = np.arange(_T, dtype=np.float64)[None, :]
    theta = np.pi * (2.0 * f + 1.0) * n / (2.0 * _T)
    fwd = np.concatenate([np.cos(theta), -np.sin(theta)], axis=0)
    inv = np.concatenate([np.cos(theta).T, -np.sin(theta).T], axis=1) / _T
    return fwd.astype(np.float32), inv.astype(np.float32)


@jax.jit(static_argnames=("A_seg_len",))
def pallas_gated_mix__memory_aug_recurrent_mem_tr__ssm_conv_h3__prompt_kernel(
    A_x: jax.Array,
    A_mem0: jax.Array,
    A_Wq: jax.Array,
    A_Wk: jax.Array,
    A_Wv: jax.Array,
    A_Wo: jax.Array,
    A_seg_len: int,
    B_q: jax.Array,
    B_k: jax.Array,
    B_v: jax.Array,
    B_shift_k: jax.Array,
    B_ssm_k: jax.Array,
    B_ssm_D: jax.Array,
    gate_w: jax.Array,
):
    del B_q
    _, S, D = A_x.shape
    _, H, DH = A_Wq.shape
    M = A_mem0.shape[1]
    SEG = int(A_seg_len)
    KS = B_shift_k.shape[1]
    L = M + SEG
    NSEG = S // SEG
    NP = H // 2
    PW = 2 * DH
    KR = -(-L // 16) * 16
    NB = S // _T
    scale = DH ** -0.5
    assert A_x.shape[0] == 1 and S % SEG == 0 and S % _T == 0 and H % 2 == 0
    assert PW % 128 == 0 and D % 128 == 0 and M % 8 == 0 and SEG % 16 == 0
    assert 2 * KR <= 128 and KS <= 8

    def kernel(x_hbm, mem0_ref, wq_hbm, wk_hbm, wv_hbm, wo_hbm, bk_hbm, bv_hbm,
               shift_ref, ssmk_hbm, ssmd_ref, gw_ref, fwd_ref, inv_ref,
               o_hbm,
               x_v, wqkv, wo_v, h_v, bpart, gate, out_v, in_sems, out_sem):

        def prologue(stage, bk_v, bv_v, ssmk_v, kpad, xf, kf):
            c_ssmk = pltpu.make_async_copy(ssmk_hbm, ssmk_v, in_sems.at[0])
            c_bk = pltpu.make_async_copy(bk_hbm, bk_v, in_sems.at[1])
            c_bv = pltpu.make_async_copy(bv_hbm, bv_v, in_sems.at[2])
            c_x = pltpu.make_async_copy(x_hbm, x_v, in_sems.at[3])
            c_w = [pltpu.make_async_copy(w, stage.at[i], in_sems.at[4 + i])
                   for i, w in enumerate((wq_hbm, wk_hbm, wv_hbm))]
            c_wo = pltpu.make_async_copy(wo_hbm, wo_v, in_sems.at[7])
            for c in (c_ssmk, c_bk, c_bv, c_x, *c_w, c_wo):
                c.start()

            fwd = fwd_ref[...].astype(BF16)
            inv = inv_ref[...].astype(BF16)

            c_ssmk.wait()
            for d in range(NB):
                kf[d] = _dot(fwd, ssmk_v[:, d * _T:(d + 1) * _T], _NT)

            c_bk.wait()
            c_bv.wait()
            taps = shift_ref[...].astype(F32)
            kpad[0:8, :] = jnp.zeros((8, D), F32)

            def fwd_block(a, carry):
                r0 = pl.multiple_of(a * _T, _T)
                kpad[8:8 + _T, :] = bk_v[pl.ds(r0, _T), :].astype(F32)
                ksh = kpad[8:8 + _T, :] * taps[0:1]
                for j in range(1, KS):
                    ksh = ksh + kpad[8 - j:8 - j + _T, :] * taps[j:j + 1]
                kpad[0:8, :] = kpad[_T:_T + 8, :]
                kv = ksh * bv_v[pl.ds(r0, _T), :].astype(F32)
                bpart[pl.ds(r0, _T), :] = kv
                xf[a] = _dot(fwd, kv.astype(BF16))
                return carry

            jax.lax.fori_loop(0, NB, fwd_block, 0)

            sub = jax.lax.broadcasted_iota(jnp.int32, (8, 128), 0)
            sign = (1 - 2 * (sub & 1)).astype(F32)

            def mac(g, carry):
                re = pl.ds(pl.multiple_of(g * 8, 8), 8)
                im = pl.ds(pl.multiple_of(_T + g * 8, 8), 8)
                for t in range(D // 128):
                    ln = slice(t * 128, (t + 1) * 128)
                    xr = [xf[a, re, ln] for a in range(NB)]
                    xi = [xf[a, im, ln] for a in range(NB)]
                    kr = [kf[a, re, ln] for a in range(NB)]
                    ki = [kf[a, im, ln] for a in range(NB)]
                    pr = pi = None
                    for c in range(NB):
                        zr = zi = None
                        for a in range(c + 1):
                            tr = xr[a] * kr[c - a] - xi[a] * ki[c - a]
                            ti = xr[a] * ki[c - a] + xi[a] * kr[c - a]
                            zr = tr if zr is None else zr + tr
                            zi = ti if zi is None else zi + ti
                        if c == 0:
                            wr, wi = zr, zi
                        else:
                            wr, wi = zr - sign * pi, zi + sign * pr
                        pr, pi = zr, zi
                        xf[c, re, ln] = wr
                        xf[c, im, ln] = wi
                return carry

            jax.lax.fori_loop(0, _T // 8, mac, 0)

            c_x.wait()
            skip = ssmd_ref[...].astype(F32).reshape(1, D)
            gw = gw_ref[...].astype(F32).reshape(1, D)

            def inv_block(c, carry):
                rows = pl.ds(pl.multiple_of(c * _T, _T), _T)
                y = _dot(inv, xf[c].astype(BF16))
                xq = x_v[rows, :].astype(F32)
                g = jax.nn.sigmoid(jnp.sum(xq * gw, axis=1, keepdims=True))
                bpart[rows, :] = (1.0 - g) * (xq * (y + bpart[rows, :] * skip))
                gate[rows, :] = jnp.broadcast_to(g, (_T, 128))
                return carry

            jax.lax.fori_loop(0, NB, inv_block, 0)

            for i in range(3):
                c_w[i].wait()

                def transpose(p, carry, i=i):
                    rows = pl.ds(pl.multiple_of(p * PW, PW), PW)
                    wqkv[p, i] = stage[i, rows, :].T
                    return carry

                jax.lax.fori_loop(0, NP, transpose, 0)
            c_wo.wait()

        pl.run_scoped(
            prologue,
            pltpu.VMEM((3, H * DH, D), BF16),
            pltpu.VMEM((S, D), BF16),
            pltpu.VMEM((S, D), BF16),
            pltpu.VMEM((D, S), BF16),
            pltpu.VMEM((_T + 8, D), F32),
            pltpu.VMEM((NB, 2 * _T, D), F32),
            pltpu.VMEM((NB, 2 * _T, D), F32),
        )

        h_v[0:M, :] = mem0_ref[...].astype(F32)

        row = jax.lax.broadcasted_iota(jnp.int32, (L, 2 * KR), 0)
        lane = jax.lax.broadcasted_iota(jnp.int32, (L, 2 * KR), 1)
        in_a = lane < KR
        col = jnp.where(in_a, lane, lane - KR)
        valid = col < L
        valid_a = valid & in_a
        valid_b = valid & (lane >= KR)
        allowed = (row < M) | (row >= col)
        dim_a = jax.lax.broadcasted_iota(jnp.int32, (L, PW), 1) < DH
        zpad = jnp.zeros((KR - L, PW), F32)

        def block_diag(t):
            a = jnp.where(dim_a, t, 0.0)
            b = jnp.where(dim_a, 0.0, t)
            return jnp.concatenate([a, zpad, b, zpad], axis=0).astype(BF16)

        def softmax(s):
            s = jnp.where(allowed, s * scale, -1e9)
            ma = jnp.max(jnp.where(valid_a, s, -jnp.inf), axis=1, keepdims=True)
            mb = jnp.max(jnp.where(valid_b, s, -jnp.inf), axis=1, keepdims=True)
            e = jnp.where(valid, jnp.exp(s - jnp.where(in_a, ma, mb)), 0.0)
            la = jnp.sum(jnp.where(in_a, e, 0.0), axis=1, keepdims=True)
            lb = jnp.sum(jnp.where(in_a, 0.0, e), axis=1, keepdims=True)
            return e * (1.0 / jnp.where(in_a, la, lb))

        def out_copy(s):
            rows = pl.ds(pl.multiple_of(s * SEG, SEG), SEG)
            return pltpu.make_async_copy(out_v.at[rows], o_hbm.at[rows], out_sem)

        def step(s, carry):
            rows = pl.ds(pl.multiple_of(s * SEG, SEG), SEG)
            h_v[M:L, :] = x_v[rows, :].astype(F32)
            h = h_v[...]
            q, k, v, p, o = {}, {}, {}, {}, {}
            acc = []

            def proj_q(i):
                q[i] = _dot(h, wqkv[i, 0])

            def proj_k(i):
                k[i] = block_diag(_dot(h, wqkv[i, 1]))

            def proj_v(i):
                v[i] = block_diag(_dot(h, wqkv[i, 2]))

            def scores(i):
                p[i] = softmax(_dot(q.pop(i), k.pop(i), _NT))

            def values(i):
                o[i] = _dot(p.pop(i), v.pop(i))

            def proj_o(i):
                y = _dot(o.pop(i), wo_v[i * PW:(i + 1) * PW, :])
                acc[:] = [y if not acc else acc[0] + y]

            held = 4
            for i in range(NP):
                proj_k(i)
                proj_q(i)
                proj_v(i)
                if i >= 1:
                    values(i - 1)
                scores(i)
                if 2 <= i < NP + 1 - held:
                    proj_o(i - 2)
            for i in range(NP - 1 - held, NP - 2):
                proj_o(i)
            values(NP - 1)
            proj_o(NP - 2)
            proj_o(NP - 1)

            y = acc[0]
            h_v[0:M, :] = y[0:M].astype(BF16).astype(F32)
            g = gate[rows, :]
            g = jnp.concatenate([g] * (D // 128), axis=1)
            out_v[rows, :] = (g * y[M:L] + bpart[rows, :]).astype(out_v.dtype)
            out_copy(s).start()
            return carry

        jax.lax.fori_loop(0, NSEG, step, 0)
        pltpu.make_async_copy(out_v, o_hbm, out_sem).wait()

    fwd_np, inv_np = _dft_matrices()
    hbm = pl.BlockSpec(memory_space=pl.ANY)
    vmem = pl.BlockSpec(memory_space=pltpu.VMEM)

    def head_major(w):
        return jnp.transpose(w, (1, 2, 0)).reshape(H * DH, D)

    out = pl.pallas_call(
        kernel,
        out_shape=jax.ShapeDtypeStruct((S, D), A_x.dtype),
        in_specs=[hbm, vmem, hbm, hbm, hbm, hbm, hbm, hbm,
                  vmem, hbm, vmem, vmem, vmem, vmem],
        out_specs=hbm,
        scratch_shapes=[
            pltpu.VMEM((S, D), BF16),
            pltpu.VMEM((NP, 3, D, PW), BF16),
            pltpu.VMEM((H * DH, D), BF16),
            pltpu.VMEM((L, D), F32),
            pltpu.VMEM((S, D), F32),
            pltpu.VMEM((S, 128), F32),
            pltpu.VMEM((S, D), A_x.dtype),
            pltpu.SemaphoreType.DMA((8,)),
            pltpu.SemaphoreType.DMA(()),
        ],
        compiler_params=pltpu.CompilerParams(vmem_limit_bytes=120 * 1024 * 1024),
    )(
        A_x.reshape(S, D), A_mem0.reshape(M, D),
        head_major(A_Wq), head_major(A_Wk), head_major(A_Wv), A_Wo.reshape(H * DH, D),
        B_k.reshape(S, D), B_v.reshape(S, D),
        B_shift_k.T, B_ssm_k, B_ssm_D, gate_w,
        jnp.asarray(fwd_np), jnp.asarray(inv_np),
    )
    return out.reshape(1, S, D)
```

```python
import numpy as np

import jax
import jax.numpy as jnp
import jax.experimental.pallas as pl
import jax.experimental.pallas.tpu as pltpu

F32 = jnp.float32
BF16 = jnp.bfloat16
U32 = jnp.uint32
_NN = (((1,), (0,)), ((), ()))
_NT = (((1,), (1,)), ((), ()))
_T = 128
_AHEAD = 8
_UNROLL = 2
_DIST = 6
_GROUP = 4
_MB, _GATES, _LEAD = 64, 2, 6


def _dot(a, b, dims=_NN):
    return jax.lax.dot_general(a, b, dims, preferred_element_type=F32)


def _dft_matrices():
    f = np.arange(_T, dtype=np.float64)[:, None]
    n = np.arange(_T, dtype=np.float64)[None, :]
    theta = np.pi * (2.0 * f + 1.0) * n / (2.0 * _T)
    fwd = np.concatenate([np.cos(theta), -np.sin(theta)], axis=0)
    inv = np.concatenate([np.cos(theta).T, -np.sin(theta).T], axis=1) / _T
    return fwd.astype(np.float32), inv.astype(np.float32)


@jax.jit(static_argnames=("A_seg_len",))
def pallas_gated_mix__memory_aug_recurrent_mem_tr__ssm_conv_h3__prompt_kernel(
    A_x: jax.Array,
    A_mem0: jax.Array,
    A_Wq: jax.Array,
    A_Wk: jax.Array,
    A_Wv: jax.Array,
    A_Wo: jax.Array,
    A_seg_len: int,
    B_q: jax.Array,
    B_k: jax.Array,
    B_v: jax.Array,
    B_shift_k: jax.Array,
    B_ssm_k: jax.Array,
    B_ssm_D: jax.Array,
    gate_w: jax.Array,
):
    del B_q
    _, S, D = A_x.shape
    _, H, DH = A_Wq.shape
    M = A_mem0.shape[1]
    SEG = int(A_seg_len)
    KS = B_shift_k.shape[1]
    L = M + SEG
    NSEG = S // SEG
    NP = H // 2
    PW = 2 * DH
    KR = -(-L // 16) * 16
    NB = S // _T
    HALF = NSEG // 2 * _AHEAD
    scale = DH ** -0.5
    assert A_x.shape[0] == 1 and S % _T == 0 and _T % SEG == 0 and H % 2 == 0
    assert PW % 128 == 0 and D % 128 == 0 and M % 8 == 0 and SEG % 16 == 0
    assert 2 * KR <= 128 and KS <= 8 and NP == NB == _T // 8 and HALF == 2 * _T

    def kernel(x_hbm, xs_hbm, mem0_ref, wq_hbm, wk_hbm, wv_hbm, wo_hbm, bk_hbm, bv_hbm,
               shift_ref, ssmk_hbm, ssmd_ref, gw_ref, fwd_ref, inv_ref,
               o_hbm,
               x_v, wq_v, wk_v, wv_v, wo_v, qa, h_v, kv_v, out_v,
               stage, bk_v, bv_v, ssmk_v, kpad, xf, kf, xa, xs_v,
               w_sems, b_sems, all_sems, xa_sem, out_sem):

        def pair_rows(p):
            return pl.ds(pl.multiple_of(p * PW, PW), PW)

        def block_rows(a):
            return pl.ds(pl.multiple_of(a * _T, _T), _T)

        def w_copy(i, p):
            src = (wq_hbm, wk_hbm, wv_hbm, wo_hbm)[i].at[pair_rows(p)]
            if i == 3:
                return pltpu.make_async_copy(src, wo_v.at[pair_rows(p)], all_sems.at[0])
            return pltpu.make_async_copy(src, stage.at[i, pair_rows(p)], w_sems.at[i, p % _DIST])

        def b_copies(a):
            blk = block_rows(a)
            return (pltpu.make_async_copy(ssmk_hbm.at[:, blk], ssmk_v.at[:, blk], b_sems.at[a]),
                    pltpu.make_async_copy(bk_hbm.at[blk], bk_v.at[blk], b_sems.at[a]),
                    pltpu.make_async_copy(bv_hbm.at[blk], bv_v.at[blk], b_sems.at[a]))

        def x_copy(a):
            blk = block_rows(a)
            return pltpu.make_async_copy(x_hbm.at[blk], x_v.at[blk], all_sems.at[1])

        def transpose(i, p):
            (wq_v, wk_v, wv_v)[i][p] = pltpu.bitcast(stage[i, pair_rows(p), :].T, U32)

        xa_copy = pltpu.make_async_copy(xs_hbm.at[:, SEG - _AHEAD:SEG, :], xs_v, xa_sem)
        xa_copy.start()
        for p in range(_UNROLL):
            w_copy(0, p).start()

        xa_copy.wait()
        for s in range(NSEG):
            r = (s % 2) * HALF + (s // 2) * _AHEAD
            xa[r:r + _AHEAD, :] = xs_v[s].astype(F32)

        def q_ahead(it, carry):
            for u in range(_UNROLL):
                w_copy(0, it * _UNROLL + u).wait()
            for u in range(_UNROLL):
                p = it * _UNROLL + u

                @pl.when(p + _UNROLL < NP)
                def _():
                    w_copy(0, p + _UNROLL).start()

                @pl.when(p + _DIST >= NP)
                def _():
                    w_copy(1, p + _DIST - NP).start()

                for c in b_copies(p):
                    c.start()
            for u in range(_UNROLL):
                p = it * _UNROLL + u
                w = stage[0, pair_rows(p), :]
                even = _dot(xa[0:HALF, :], w, _NT)
                odd = _dot(xa[HALF:2 * HALF, :], w, _NT)
                qa[p] = pltpu.pack_elementwise([even, odd], packed_dtype=BF16)
                transpose(0, p)
            return carry

        jax.lax.fori_loop(0, NP // _UNROLL, q_ahead, 0)

        fwd = fwd_ref[...].astype(BF16)
        taps = shift_ref[...].astype(F32)
        kpad[0:8, :] = jnp.zeros((8, D), F32)

        def spectra(it, carry):
            for u in range(_UNROLL):
                a = it * _UNROLL + u
                for c in b_copies(a):
                    c.wait()
                w_copy(1, a).wait()
            for u in range(_UNROLL):
                a = it * _UNROLL + u

                @pl.when(a + _DIST < NP)
                def _():
                    w_copy(1, a + _DIST).start()

                @pl.when(a + _DIST >= NP)
                def _():
                    w_copy(2, a + _DIST - NP).start()

            for u in range(_UNROLL):
                a = it * _UNROLL + u
                blk = block_rows(a)
                kf[a] = _dot(fwd, ssmk_v[:, blk], _NT)
                kpad[8:8 + _T, :] = bk_v[blk, :].astype(F32)
                ksh = kpad[8:8 + _T, :] * taps[0:1]
                for j in range(1, KS):
                    ksh = ksh + kpad[8 - j:8 - j + _T, :] * taps[j:j + 1]
                kpad[0:8, :] = kpad[_T:_T + 8, :]
                kv = (ksh * bv_v[blk, :].astype(F32)).astype(BF16)
                kv_v[blk, :] = kv
                xf[a, :, 0:D] = _dot(fwd, kv)
                transpose(1, a)
            return carry

        jax.lax.fori_loop(0, NB // _UNROLL, spectra, 0)

        sub = jax.lax.broadcasted_iota(jnp.int32, (8, 128), 0)
        sign = (1 - 2 * (sub & 1)).astype(F32)

        def block_products(g):
            re = pl.ds(pl.multiple_of(g * 8, 8), 8)
            im = pl.ds(pl.multiple_of(_T + g * 8, 8), 8)
            for t in range(D // 128):
                ln = slice(t * 128, (t + 1) * 128)
                above = None
                for top in range(NB - 1, -1, -_GROUP):
                    z = {}
                    for a in range(top + 1):
                        xr, xi = xf[a, re, ln], xf[a, im, ln]
                        for c in range(top, max(top - _GROUP, a - 1), -1):
                            kr, ki = kf[c - a, re, ln], kf[c - a, im, ln]
                            tr, ti = xr * kr - xi * ki, xr * ki + xi * kr
                            z[c] = (tr, ti) if a == 0 else (z[c][0] + tr, z[c][1] + ti)
                            yield
                    for c in range(top, top - _GROUP, -1):
                        if above is not None:
                            xf[c + 1, re, ln] = above[0] - sign * z[c][1]
                            xf[c + 1, im, ln] = above[1] + sign * z[c][0]
                        above = z[c]
                xf[0, re, ln], xf[0, im, ln] = above

        def products(g, carry):
            w_copy(2, g).wait()

            @pl.when(g + _DIST < NP)
            def _():
                w_copy(2, g + _DIST).start()

            w_copy(3, g).start()
            x_copy(g).start()

            work = block_products(g)
            pieces = [(t, m) for t in range(PW // 128) for m in range(0, HALF, _MB)]
            slots = len(pieces) * 2 * _GATES + _LEAD
            total = (D // 128) * NB * (NB + 1) // 2
            done = [0, 0]

            def pace():
                done[0] += 1
                while done[1] < total * done[0] // slots:
                    next(work)
                    done[1] += 1

            for _ in range(_LEAD):
                pace()
            for n, (t, m) in enumerate(pieces):
                w = pltpu.bitcast(wk_v[g, :, t * 128:(t + 1) * 128], BF16)
                cols = slice(D + t * 128, D + (t + 1) * 128)
                halves = []
                for base in (0, HALF):
                    y = _dot(xa[base + m:base + m + _MB, :], w)
                    for r in range(0, _MB, _MB // _GATES):
                        xf[g, m + r:m + r + 8, cols] = y[r:r + 8]
                        pace()
                    halves.append(y)
                xf[g, m:m + _MB, cols] = pltpu.bitcast(
                    pltpu.pack_elementwise(halves, packed_dtype=BF16), F32)
            for _ in work:
                pass
            transpose(2, g)
            return carry

        jax.lax.fori_loop(0, NP, products, 0)
        pltpu.make_async_copy(wo_hbm, wo_v, all_sems.at[0]).wait()
        pltpu.make_async_copy(x_hbm, x_v, all_sems.at[1]).wait()

        skip = ssmd_ref[...].astype(F32).reshape(1, D)
        gw = gw_ref[...].astype(F32).reshape(1, D)
        h_v[0:M, :] = mem0_ref[...].astype(F32)

        row = jax.lax.broadcasted_iota(jnp.int32, (L, 2 * KR), 0)
        lane = jax.lax.broadcasted_iota(jnp.int32, (L, 2 * KR), 1)
        in_a = lane < KR
        col = jnp.where(in_a, lane, lane - KR)
        valid = col < L
        valid_a = valid & in_a
        valid_b = valid & (lane >= KR)
        allowed = (row < M) | (row >= col)
        dim_a = jax.lax.broadcasted_iota(jnp.int32, (L, PW), 1) < DH
        zpad = jnp.zeros((KR - L, PW), F32)

        def block_diag(t):
            a = jnp.where(dim_a, t, 0.0)
            b = jnp.where(dim_a, 0.0, t)
            return jnp.concatenate([a, zpad, b, zpad], axis=0).astype(BF16)

        def softmax(s):
            s = jnp.where(allowed, s * scale, -1e9)
            ma = jnp.max(jnp.where(valid_a, s, -jnp.inf), axis=1, keepdims=True)
            mb = jnp.max(jnp.where(valid_b, s, -jnp.inf), axis=1, keepdims=True)
            e = jnp.where(valid, jnp.exp(s - jnp.where(in_a, ma, mb)), 0.0)
            la = jnp.sum(jnp.where(in_a, e, 0.0), axis=1, keepdims=True)
            lb = jnp.sum(jnp.where(in_a, 0.0, e), axis=1, keepdims=True)
            return e * (1.0 / jnp.where(in_a, la, lb))

        def step(s, carry):
            rows = pl.ds(pl.multiple_of(s * SEG, SEG), SEG)
            xq = x_v[rows, :].astype(F32)
            h_v[M:L, :] = xq
            h = h_v[...]
            ahead = pl.ds(pl.multiple_of((s // 2) * _AHEAD, _AHEAD), _AHEAD)
            ahead_shift = ((1 - (s & 1)) * 16).astype(U32)
            q, k, v, p, o = {}, {}, {}, {}, {}
            acc = []

            def project(i, j):
                w = pltpu.bitcast((wq_v, wk_v, wv_v)[j][i], BF16)
                if j == 2:
                    return _dot(h, w)
                word = qa[i, ahead, :] if j == 0 else pltpu.bitcast(xf[i, ahead, D:D + PW], U32)
                tail = pltpu.bitcast((word << ahead_shift) & U32(0xFFFF0000), F32)
                return jnp.concatenate([_dot(h[0:L - _AHEAD], w), tail], axis=0)

            def proj_o(i):
                y = _dot(o.pop(i), wo_v[i * PW:(i + 1) * PW, :])
                acc[:] = [y if not acc else acc[0] + y]

            blk, part = s // (_T // SEG), s % (_T // SEG)
            conv = _dot(inv_ref[pl.ds(pl.multiple_of(part * SEG, SEG), SEG), :],
                        xf[blk, :, 0:D].astype(BF16))
            g = jax.nn.sigmoid(jnp.sum(xq * gw, axis=1, keepdims=True))
            b = (1.0 - g) * (xq * (conv + kv_v[rows, :].astype(F32) * skip))

            held = 4
            for i in range(NP):
                k[i] = block_diag(project(i, 1))
                q[i] = project(i, 0)
                v[i] = block_diag(project(i, 2))
                if i >= 1:
                    o[i - 1] = _dot(p.pop(i - 1), v.pop(i - 1))
                p[i] = softmax(_dot(q.pop(i), k.pop(i), _NT))
                if 2 <= i < NP + 1 - held:
                    proj_o(i - 2)
            for i in range(NP - 1 - held, NP - 2):
                proj_o(i)
            o[NP - 1] = _dot(p.pop(NP - 1), v.pop(NP - 1))
            proj_o(NP - 2)
            proj_o(NP - 1)

            y = acc[0]
            h_v[0:M, :] = y[0:M].astype(BF16).astype(F32)
            out_v[rows, :] = (g * y[M:L] + b).astype(out_v.dtype)
            pltpu.make_async_copy(out_v.at[rows], o_hbm.at[rows], out_sem).start()
            return carry

        jax.lax.fori_loop(0, NSEG, step, 0, unroll=4)
        pltpu.make_async_copy(out_v, o_hbm, out_sem).wait()

    fwd_np, inv_np = _dft_matrices()
    hbm = pl.BlockSpec(memory_space=pl.ANY)
    vmem = pl.BlockSpec(memory_space=pltpu.VMEM)

    def head_major(w):
        return jnp.transpose(w, (1, 2, 0)).reshape(H * DH, D)

    out = pl.pallas_call(
        kernel,
        out_shape=jax.ShapeDtypeStruct((S, D), A_x.dtype),
        in_specs=[hbm, hbm, vmem, hbm, hbm, hbm, hbm, hbm, hbm,
                  vmem, hbm, vmem, vmem, vmem, vmem],
        out_specs=hbm,
        scratch_shapes=[
            pltpu.VMEM((S, D), BF16),
            pltpu.VMEM((NP, D // 2, PW), U32),
            pltpu.VMEM((NP, D // 2, PW), U32),
            pltpu.VMEM((NP, D // 2, PW), U32),
            pltpu.VMEM((H * DH, D), BF16),
            pltpu.VMEM((NP, HALF, PW), U32),
            pltpu.VMEM((L, D), F32),
            pltpu.VMEM((S, D), BF16),
            pltpu.VMEM((S, D), A_x.dtype),
            pltpu.VMEM((3, H * DH, D), BF16),
            pltpu.VMEM((S, D), BF16),
            pltpu.VMEM((S, D), BF16),
            pltpu.VMEM((D, S), BF16),
            pltpu.VMEM((_T + 8, D), F32),
            pltpu.VMEM((NB, 2 * _T, D + PW), F32),
            pltpu.VMEM((NB, 2 * _T, D), F32),
            pltpu.VMEM((2 * HALF, D), F32),
            pltpu.VMEM((NSEG, _AHEAD, D), BF16),
            pltpu.SemaphoreType.DMA((3, _DIST)),
            pltpu.SemaphoreType.DMA((NB,)),
            pltpu.SemaphoreType.DMA((2,)),
            pltpu.SemaphoreType.DMA(()),
            pltpu.SemaphoreType.DMA(()),
        ],
        compiler_params=pltpu.CompilerParams(vmem_limit_bytes=124 * 1024 * 1024),
    )(
        A_x.reshape(S, D), A_x.reshape(NSEG, SEG, D), A_mem0.reshape(M, D),
        head_major(A_Wq), head_major(A_Wk), head_major(A_Wv), A_Wo.reshape(H * DH, D),
        B_k.reshape(S, D), B_v.reshape(S, D),
        B_shift_k.T, B_ssm_k, B_ssm_D, gate_w,
        jnp.asarray(fwd_np), jnp.asarray(inv_np),
    )
    return out.reshape(1, S, D)
```

```python
import numpy as np

import jax
import jax.numpy as jnp
import jax.experimental.pallas as pl
import jax.experimental.pallas.tpu as pltpu

F32 = jnp.float32
BF16 = jnp.bfloat16
U32 = jnp.uint32
_NN = (((1,), (0,)), ((), ()))
_NT = (((1,), (1,)), ((), ()))
_T = 128
_AHEAD = 8
_DIST = 2
_SLOTS = 4
_GROUP = 4
_MB, _GATES, _LEAD = 64, 2, 6
_HELD = 4


def _dot(a, b, dims=_NN):
    return jax.lax.dot_general(a, b, dims, preferred_element_type=F32)


def _dft_matrices():
    f = np.arange(_T, dtype=np.float64)[:, None]
    n = np.arange(_T, dtype=np.float64)[None, :]
    theta = np.pi * (2.0 * f + 1.0) * n / (2.0 * _T)
    fwd = np.concatenate([np.cos(theta), -np.sin(theta)], axis=0)
    inv = np.concatenate([np.cos(theta).T, -np.sin(theta).T], axis=1) / _T
    return fwd.astype(np.float32), inv.astype(np.float32)


@jax.jit(static_argnames=("A_seg_len",))
def pallas_gated_mix__memory_aug_recurrent_mem_tr__ssm_conv_h3__prompt_kernel(
    A_x: jax.Array,
    A_mem0: jax.Array,
    A_Wq: jax.Array,
    A_Wk: jax.Array,
    A_Wv: jax.Array,
    A_Wo: jax.Array,
    A_seg_len: int,
    B_q: jax.Array,
    B_k: jax.Array,
    B_v: jax.Array,
    B_shift_k: jax.Array,
    B_ssm_k: jax.Array,
    B_ssm_D: jax.Array,
    gate_w: jax.Array,
):
    del B_q
    _, S, D = A_x.shape
    _, H, DH = A_Wq.shape
    M = A_mem0.shape[1]
    SEG = int(A_seg_len)
    KS = B_shift_k.shape[1]
    L = M + SEG
    NSEG = S // SEG
    NP = H // 2
    PW = 2 * DH
    KR = -(-L // 16) * 16
    NB = S // _T
    SPB = _T // SEG
    HALF = NSEG // 2 * _AHEAD
    scale = DH ** -0.5
    assert A_x.shape[0] == 1 and S % _T == 0 and _T % (2 * SEG) == 0 and H % 2 == 0
    assert PW % 128 == 0 and D % 128 == 0 and M % 8 == 0 and SEG % 16 == 0
    assert 2 * KR <= 128 and KS <= 8 and NP == NB == _T // 8 and HALF == 2 * _T

    def kernel(x_hbm, xs_hbm, mem0_ref, wq_hbm, wk_hbm, wv_hbm, wo_hbm, bk_hbm, bv_hbm,
               shift_ref, ssmk_hbm, ssmd_ref, gw_ref, fwd_ref, inv_ref,
               o_hbm,
               x_v, wq_v, wk_v, wv_v, wo_v, h_v, kv_v, out_v,
               stage, bk_v, bv_v, ssmk_v, kpad, xf, kf, xa, xs_v,
               w_sems, b_sems, xs_sem, wo_sem, x_sem, out_sem):
        qkv_v = (wq_v, wk_v, wv_v)

        def pair_rows(p):
            return pl.ds(pl.multiple_of(p * PW, PW), PW)

        def block_rows(a):
            return pl.ds(pl.multiple_of(a * _T, _T), _T)

        def w_copy(j, p):
            src = (wq_hbm, wk_hbm, wv_hbm)[j]
            return pltpu.make_async_copy(
                src.at[pair_rows(p)], stage.at[j, pair_rows(p)], w_sems.at[j, p % _SLOTS])

        def wo_copy(p):
            return pltpu.make_async_copy(wo_hbm.at[pair_rows(p)], wo_v.at[pair_rows(p)], wo_sem)

        def b_copies(a):
            blk, sem = block_rows(a), b_sems.at[a % _SLOTS]
            return (pltpu.make_async_copy(ssmk_hbm.at[:, blk], ssmk_v.at[:, blk], sem),
                    pltpu.make_async_copy(bk_hbm.at[blk], bk_v.at[blk], sem),
                    pltpu.make_async_copy(bv_hbm.at[blk], bv_v.at[blk], sem))

        def x_copy(a):
            return pltpu.make_async_copy(x_hbm.at[block_rows(a)], x_v.at[block_rows(a)], x_sem)

        def start_first_phase_copies(a):
            for c in b_copies(a):
                c.start()
            w_copy(0, a).start()
            w_copy(1, a).start()

        def transpose(j, p):
            qkv_v[j][p] = pltpu.bitcast(stage[j, pair_rows(p), :].T, U32)

        def ahead_lanes(j, t):
            return slice(D + j * PW + t * 128, D + j * PW + (t + 1) * 128)

        def pack_segments(even, odd):
            return pltpu.bitcast(pltpu.pack_elementwise([even, odd], packed_dtype=BF16), F32)

        xs_copy = pltpu.make_async_copy(xs_hbm.at[:, SEG - _AHEAD:SEG, :], xs_v, xs_sem)
        xs_copy.start()
        start_first_phase_copies(0)
        xs_copy.wait()
        for a in range(1, _DIST):
            start_first_phase_copies(a)
        for s in range(NSEG):
            r = (s % 2) * HALF + (s // 2) * _AHEAD
            xa[r:r + _AHEAD, :] = xs_v[s].astype(F32)
        fwd = fwd_ref[...]
        taps = shift_ref[...].astype(F32)
        kpad[0:8, :] = jnp.zeros((8, D), F32)

        def spectra(a, carry):
            for c in b_copies(a):
                c.wait()
            w_copy(0, a).wait()
            w_copy(1, a).wait()

            @pl.when(a + _DIST < NB)
            def _():
                start_first_phase_copies(a + _DIST)

            @pl.when(a + _DIST >= NB)
            def _():
                w_copy(2, a + _DIST - NB).start()
                wo_copy(a + _DIST - NB).start()

            blk = block_rows(a)
            kf[a] = _dot(fwd, ssmk_v[:, blk], _NT)
            kpad[8:8 + _T, :] = bk_v[blk, :].astype(F32)
            ksh = kpad[8:8 + _T, :] * taps[0:1]
            for j in range(1, KS):
                ksh = ksh + kpad[8 - j:8 - j + _T, :] * taps[j:j + 1]
            kpad[0:8, :] = kpad[_T:_T + 8, :]
            kv = (ksh * bv_v[blk, :].astype(F32)).astype(BF16)
            kv_v[blk, :] = kv
            for t in range(PW // 128):
                w = stage[0, pl.ds(pl.multiple_of(a * PW + t * 128, 128), 128), :]
                xf[a, :, ahead_lanes(0, t)] = pack_segments(
                    _dot(xa[0:HALF, :], w, _NT), _dot(xa[HALF:2 * HALF, :], w, _NT))
                if t == 0:
                    xf[a, :, 0:D] = _dot(fwd, kv)
                if t == 1:
                    transpose(1, a)
                    spare = pl.ds(pl.multiple_of(2 * HALF + 8 * (a >> 20), 8), 8)
                    xa[spare, 0:128] = pltpu.bitcast(wk_v[a, D // 2 - 8:D // 2, PW - 128:PW], F32)
            transpose(0, a)
            return carry

        jax.lax.fori_loop(0, NB, spectra, 0)

        sub = jax.lax.broadcasted_iota(jnp.int32, (8, 128), 0)
        sign = (1 - 2 * (sub & 1)).astype(F32)

        def block_products(g):
            re = pl.ds(pl.multiple_of(g * 8, 8), 8)
            im = pl.ds(pl.multiple_of(_T + g * 8, 8), 8)
            for t in range(D // 128):
                ln = slice(t * 128, (t + 1) * 128)
                above = None
                for top in range(NB - 1, -1, -_GROUP):
                    z = {}
                    for a in range(top + 1):
                        xr, xi = xf[a, re, ln], xf[a, im, ln]
                        for c in range(top, max(top - _GROUP, a - 1), -1):
                            kr, ki = kf[c - a, re, ln], kf[c - a, im, ln]
                            tr, ti = xr * kr - xi * ki, xr * ki + xi * kr
                            z[c] = (tr, ti) if a == 0 else (z[c][0] + tr, z[c][1] + ti)
                            yield
                    for c in range(top, top - _GROUP, -1):
                        if above is not None:
                            xf[c + 1, re, ln] = above[0] - sign * z[c][1]
                            xf[c + 1, im, ln] = above[1] + sign * z[c][0]
                        above = z[c]
                xf[0, re, ln], xf[0, im, ln] = above

        def products(g, carry):
            w_copy(2, g).wait()

            @pl.when(g + _DIST < NP)
            def _():
                w_copy(2, g + _DIST).start()
                wo_copy(g + _DIST).start()

            @pl.when(g + _DIST == NP)
            def _():
                x_copy(0).start()

            work = block_products(g)
            pieces = [(t, m) for t in range(PW // 128) for m in range(0, HALF, _MB)]
            slots = len(pieces) * 2 * _GATES + _LEAD
            total = (D // 128) * NB * (NB + 1) // 2
            used = [0, 0]

            def pace():
                used[0] += 1
                while used[1] < total * used[0] // slots:
                    next(work)
                    used[1] += 1

            for _ in range(_LEAD):
                pace()
            for t, m in pieces:
                w = pltpu.bitcast(wk_v[g, :, t * 128:(t + 1) * 128], BF16)
                halves = []
                for base in (0, HALF):
                    y = _dot(xa[base + m:base + m + _MB, :], w)
                    for r in range(0, _MB, _MB // _GATES):
                        xf[g, m + r:m + r + 8, ahead_lanes(1, t)] = y[r:r + 8]
                        pace()
                    halves.append(y)
                xf[g, m:m + _MB, ahead_lanes(1, t)] = pack_segments(*halves)
            for _ in work:
                pass
            transpose(2, g)
            return carry

        jax.lax.fori_loop(0, NP, products, 0)
        pltpu.make_async_copy(wo_hbm, wo_v, wo_sem).wait()

        skip = ssmd_ref[...].astype(F32).reshape(1, D)
        gw = gw_ref[...].astype(F32).reshape(1, D)
        h_v[0:M, :] = mem0_ref[...].astype(F32)

        row = jax.lax.broadcasted_iota(jnp.int32, (L, 2 * KR), 0)
        lane = jax.lax.broadcasted_iota(jnp.int32, (L, 2 * KR), 1)
        in_a = lane < KR
        col = jnp.where(in_a, lane, lane - KR)
        valid = col < L
        valid_a = valid & in_a
        valid_b = valid & (lane >= KR)
        allowed = (row < M) | (row >= col)
        dim_a = jax.lax.broadcasted_iota(jnp.int32, (L, PW), 1) < DH
        zpad = jnp.zeros((KR - L, PW), F32)

        def block_diag(t):
            a = jnp.where(dim_a, t, 0.0)
            b = jnp.where(dim_a, 0.0, t)
            return jnp.concatenate([a, zpad, b, zpad], axis=0).astype(BF16)

        def softmax(s):
            s = jnp.where(allowed, s * scale, -1e9)
            ma = jnp.max(jnp.where(valid_a, s, -jnp.inf), axis=1, keepdims=True)
            mb = jnp.max(jnp.where(valid_b, s, -jnp.inf), axis=1, keepdims=True)
            e = jnp.where(valid, jnp.exp(s - jnp.where(in_a, ma, mb)), 0.0)
            la = jnp.sum(jnp.where(in_a, e, 0.0), axis=1, keepdims=True)
            lb = jnp.sum(jnp.where(in_a, 0.0, e), axis=1, keepdims=True)
            return e * (1.0 / jnp.where(in_a, la, lb))

        def step(blk, part):
            rows = pl.ds(pl.multiple_of(blk * _T + part * SEG, SEG), SEG)
            ahead = pl.ds(pl.multiple_of((blk * (SPB // 2) + part // 2) * _AHEAD, _AHEAD), _AHEAD)
            xq = x_v[rows, :].astype(F32)
            h_v[M:L, :] = xq
            h = h_v[...]
            q, k, v, p, o = {}, {}, {}, {}, {}
            acc = []

            def project(i, j):
                w = pltpu.bitcast(qkv_v[j][i], BF16)
                if j == 2:
                    return _dot(h, w)
                word = pltpu.bitcast(xf[i, ahead, D + j * PW:D + (j + 1) * PW], U32)
                tail = word & U32(0xFFFF0000) if part % 2 else word << U32(16)
                return jnp.concatenate(
                    [_dot(h[0:L - _AHEAD], w), pltpu.bitcast(tail, F32)], axis=0)

            def project_out(i):
                y = _dot(o.pop(i), wo_v[i * PW:(i + 1) * PW, :])
                acc[:] = [y if not acc else acc[0] + y]

            conv = _dot(inv_ref[part * SEG:(part + 1) * SEG, :], xf[blk, :, 0:D].astype(BF16))
            g = jax.nn.sigmoid(jnp.sum(xq * gw, axis=1, keepdims=True))
            b = (1.0 - g) * (xq * (conv + kv_v[rows, :].astype(F32) * skip))

            for i in range(NP):
                k[i] = block_diag(project(i, 1))
                q[i] = project(i, 0)
                v[i] = block_diag(project(i, 2))
                if i >= 1:
                    o[i - 1] = _dot(p.pop(i - 1), v.pop(i - 1))
                p[i] = softmax(_dot(q.pop(i), k.pop(i), _NT))
                if 2 <= i < NP + 1 - _HELD:
                    project_out(i - 2)
            for i in range(NP - 1 - _HELD, NP - 2):
                project_out(i)
            o[NP - 1] = _dot(p.pop(NP - 1), v.pop(NP - 1))
            project_out(NP - 2)
            project_out(NP - 1)

            y = acc[0]
            h_v[0:M, :] = y[0:M].astype(BF16).astype(F32)
            out_v[rows, :] = (g * y[M:L] + b).astype(out_v.dtype)
            pltpu.make_async_copy(out_v.at[rows], o_hbm.at[rows], out_sem).start()

        def block(blk, carry):
            x_copy(blk).wait()

            @pl.when(blk + 1 < NB)
            def _():
                x_copy(blk + 1).start()

            for part in range(SPB):
                step(blk, part)
            return carry

        jax.lax.fori_loop(0, NB, block, 0)
        pltpu.make_async_copy(out_v, o_hbm, out_sem).wait()

    fwd_np, inv_np = _dft_matrices()
    hbm = pl.BlockSpec(memory_space=pl.ANY)
    vmem = pl.BlockSpec(memory_space=pltpu.VMEM)

    def head_major(w):
        return jnp.transpose(w, (1, 2, 0)).reshape(H * DH, D)

    out = pl.pallas_call(
        kernel,
        out_shape=jax.ShapeDtypeStruct((S, D), A_x.dtype),
        in_specs=[hbm, hbm, vmem, hbm, hbm, hbm, hbm, hbm, hbm,
                  vmem, hbm, vmem, vmem, vmem, vmem],
        out_specs=hbm,
        scratch_shapes=[
            pltpu.VMEM((S, D), BF16),
            pltpu.VMEM((NP, D // 2, PW), U32),
            pltpu.VMEM((NP, D // 2, PW), U32),
            pltpu.VMEM((NP, D // 2, PW), U32),
            pltpu.VMEM((H * DH, D), BF16),
            pltpu.VMEM((L, D), F32),
            pltpu.VMEM((S, D), BF16),
            pltpu.VMEM((S, D), A_x.dtype),
            pltpu.VMEM((3, H * DH, D), BF16),
            pltpu.VMEM((S, D), BF16),
            pltpu.VMEM((S, D), BF16),
            pltpu.VMEM((D, S), BF16),
            pltpu.VMEM((_T + 8, D), F32),
            pltpu.VMEM((NB, 2 * _T, D + 2 * PW), F32),
            pltpu.VMEM((NB, 2 * _T, D), F32),
            pltpu.VMEM((2 * HALF + 8, D), F32),
            pltpu.VMEM((NSEG, _AHEAD, D), BF16),
            pltpu.SemaphoreType.DMA((3, _SLOTS)),
            pltpu.SemaphoreType.DMA((_SLOTS,)),
            pltpu.SemaphoreType.DMA(()),
            pltpu.SemaphoreType.DMA(()),
            pltpu.SemaphoreType.DMA(()),
            pltpu.SemaphoreType.DMA(()),
        ],
        compiler_params=pltpu.CompilerParams(vmem_limit_bytes=124 * 1024 * 1024),
    )(
        A_x.reshape(S, D), A_x.reshape(NSEG, SEG, D), A_mem0.reshape(M, D),
        head_major(A_Wq), head_major(A_Wk), head_major(A_Wv), A_Wo.reshape(H * DH, D),
        B_k.reshape(S, D), B_v.reshape(S, D),
        B_shift_k.T, B_ssm_k, B_ssm_D, gate_w,
        jnp.asarray(fwd_np.astype(BF16)), jnp.asarray(inv_np),
    )
    return out.reshape(1, S, D)
```

```python
import numpy as np

import jax
import jax.numpy as jnp
import jax.experimental.pallas as pl
import jax.experimental.pallas.tpu as pltpu

F32 = jnp.float32
BF16 = jnp.bfloat16
U32 = jnp.uint32
_NN = (((1,), (0,)), ((), ()))
_NT = (((1,), (1,)), ((), ()))
_T = 128
_AHEAD = 8
_DIST = 2
_SLOTS = 4
_GROUP = 4
_MB, _GATES, _LEAD = 64, (0, 32), 6
_HELD = 4


def _dot(a, b, dims=_NN):
    return jax.lax.dot_general(a, b, dims, preferred_element_type=F32)


def _dft_matrices():
    f = np.arange(_T, dtype=np.float64)[:, None]
    n = np.arange(_T, dtype=np.float64)[None, :]
    theta = np.pi * (2.0 * f + 1.0) * n / (2.0 * _T)
    fwd = np.concatenate([np.cos(theta), -np.sin(theta)], axis=0)
    inv = np.concatenate([np.cos(theta).T, -np.sin(theta).T], axis=1) / _T
    return fwd.astype(np.float32), inv.astype(np.float32)


@jax.jit(static_argnames=("A_seg_len",))
def pallas_gated_mix__memory_aug_recurrent_mem_tr__ssm_conv_h3__prompt_kernel(
    A_x: jax.Array,
    A_mem0: jax.Array,
    A_Wq: jax.Array,
    A_Wk: jax.Array,
    A_Wv: jax.Array,
    A_Wo: jax.Array,
    A_seg_len: int,
    B_q: jax.Array,
    B_k: jax.Array,
    B_v: jax.Array,
    B_shift_k: jax.Array,
    B_ssm_k: jax.Array,
    B_ssm_D: jax.Array,
    gate_w: jax.Array,
):
    del B_q
    _, S, D = A_x.shape
    _, H, DH = A_Wq.shape
    M = A_mem0.shape[1]
    SEG = int(A_seg_len)
    KS = B_shift_k.shape[1]
    L = M + SEG
    NSEG = S // SEG
    NP = H // 2
    PW = 2 * DH
    KR = -(-L // 16) * 16
    NB = S // _T
    SPB = _T // SEG
    HALF = NSEG // 2 * _AHEAD
    scale = DH ** -0.5
    assert A_x.shape[0] == 1 and S % _T == 0 and _T % (2 * SEG) == 0 and H % 2 == 0
    assert PW % 128 == 0 and D % 128 == 0 and M % 8 == 0 and SEG % 16 == 0
    assert 2 * KR <= 128 and KS <= 8 and NP == NB == _T // 8 and HALF == 2 * _T

    def kernel(x_hbm, xs_hbm, mem0_ref, wq_hbm, wk_hbm, wv_hbm, wo_hbm, bk_hbm, bv_hbm,
               shift_ref, ssmk_hbm, ssmd_ref, gw_ref, fwd_ref, inv_ref,
               o_hbm,
               x_v, wq_v, wk_v, wv_v, wo_v, h_v, kv_v, out_v,
               stage, bk_v, bv_v, ssmk_v, kpad, xf, kf, xa, xs_v,
               w_sems, b_sems, xs_sem, wo_sem, x_sem, out_sem):
        qkv_v = (wq_v, wk_v, wv_v)

        def pair_rows(p):
            return pl.ds(pl.multiple_of(p * PW, PW), PW)

        def block_rows(a):
            return pl.ds(pl.multiple_of(a * _T, _T), _T)

        def w_copy(j, p):
            src = (wq_hbm, wk_hbm, wv_hbm)[j]
            return pltpu.make_async_copy(
                src.at[pair_rows(p)], stage.at[j, pair_rows(p)], w_sems.at[j, p % _SLOTS])

        def wo_copy(p):
            return pltpu.make_async_copy(wo_hbm.at[pair_rows(p)], wo_v.at[pair_rows(p)], wo_sem)

        def b_copies(a):
            blk, sem = block_rows(a), b_sems.at[a % _SLOTS]
            return (pltpu.make_async_copy(ssmk_hbm.at[:, blk], ssmk_v.at[:, blk], sem),
                    pltpu.make_async_copy(bk_hbm.at[blk], bk_v.at[blk], sem),
                    pltpu.make_async_copy(bv_hbm.at[blk], bv_v.at[blk], sem))

        def x_copy(a):
            return pltpu.make_async_copy(x_hbm.at[block_rows(a)], x_v.at[block_rows(a)], x_sem)

        def start_first_phase_copies(a):
            for c in b_copies(a):
                c.start()
            w_copy(0, a).start()
            w_copy(1, a).start()

        def transpose(j, p):
            qkv_v[j][p] = pltpu.bitcast(stage[j, pair_rows(p), :].T, U32)

        def ahead_lanes(j, t):
            return slice(D + j * PW + t * 128, D + j * PW + (t + 1) * 128)

        def pack_segments(y):
            return pltpu.bitcast(y.astype(BF16), F32)

        xs_copy = pltpu.make_async_copy(xs_hbm.at[:, SEG - _AHEAD:SEG, :], xs_v, xs_sem)
        xs_copy.start()
        start_first_phase_copies(0)
        xs_copy.wait()
        for a in range(1, _DIST):
            start_first_phase_copies(a)
        for s in range(0, NSEG, 2):
            even, odd = (pltpu.bitcast(xs_v[s + i].astype(F32), U32) for i in range(2))
            xa[s * _AHEAD:(s + 2) * _AHEAD, :] = pltpu.bitcast((even >> U32(16)) | odd, BF16).astype(F32)
        fwd = fwd_ref[...]
        taps = shift_ref[...].astype(F32)
        kpad[0:8, :] = jnp.zeros((8, D), F32)

        def spectra(a, carry):
            for c in b_copies(a):
                c.wait()
            w_copy(0, a).wait()
            w_copy(1, a).wait()

            @pl.when(a + _DIST < NB)
            def _():
                start_first_phase_copies(a + _DIST)

            @pl.when(a + _DIST >= NB)
            def _():
                w_copy(2, a + _DIST - NB).start()
                wo_copy(a + _DIST - NB).start()

            blk = block_rows(a)
            kf[a] = _dot(fwd, ssmk_v[:, blk], _NT)
            kpad[8:8 + _T, :] = bk_v[blk, :].astype(F32)
            ksh = kpad[8:8 + _T, :] * taps[0:1]
            for j in range(1, KS):
                ksh = ksh + kpad[8 - j:8 - j + _T, :] * taps[j:j + 1]
            kpad[0:8, :] = kpad[_T:_T + 8, :]
            kv = (ksh * bv_v[blk, :].astype(F32)).astype(BF16)
            kv_v[blk, :] = kv
            for t in range(PW // 128):
                w = stage[0, pl.ds(pl.multiple_of(a * PW + t * 128, 128), 128), :]
                for m in (0, HALF):
                    xf[a, m // 2:(m + HALF) // 2, ahead_lanes(0, t)] = pack_segments(
                        _dot(xa[m:m + HALF, :], w, _NT))
                if t == 0:
                    xf[a, :, 0:D] = _dot(fwd, kv)
                if t == 1:
                    transpose(1, a)
                    spare = pl.ds(pl.multiple_of(2 * HALF + 8 * (a >> 20), 8), 8)
                    xa[spare, 0:128] = pltpu.bitcast(wk_v[a, D // 2 - 8:D // 2, PW - 128:PW], F32)
            transpose(0, a)
            return carry

        jax.lax.fori_loop(0, NB, spectra, 0)

        sub = jax.lax.broadcasted_iota(jnp.int32, (8, 128), 0)
        sign = (1 - 2 * (sub & 1)).astype(F32)

        def block_products(g):
            re = pl.ds(pl.multiple_of(g * 8, 8), 8)
            im = pl.ds(pl.multiple_of(_T + g * 8, 8), 8)
            for t in range(D // 128):
                ln = slice(t * 128, (t + 1) * 128)
                above = None
                for top in range(NB - 1, -1, -_GROUP):
                    z = {}
                    for a in range(top + 1):
                        xr, xi = xf[a, re, ln], xf[a, im, ln]
                        for c in range(top, max(top - _GROUP, a - 1), -1):
                            kr, ki = kf[c - a, re, ln], kf[c - a, im, ln]
                            tr, ti = xr * kr - xi * ki, xr * ki + xi * kr
                            z[c] = (tr, ti) if a == 0 else (z[c][0] + tr, z[c][1] + ti)
                            yield
                    for c in range(top, top - _GROUP, -1):
                        if above is not None:
                            xf[c + 1, re, ln] = above[0] - sign * z[c][1]
                            xf[c + 1, im, ln] = above[1] + sign * z[c][0]
                        above = z[c]
                xf[0, re, ln], xf[0, im, ln] = above

        def products(g, carry):
            w_copy(2, g).wait()

            @pl.when(g + _DIST < NP)
            def _():
                w_copy(2, g + _DIST).start()
                wo_copy(g + _DIST).start()

            @pl.when(g + _DIST == NP)
            def _():
                x_copy(0).start()

            work = block_products(g)
            pieces = [(t, m) for t in range(PW // 128) for m in range(0, 2 * HALF, _MB)]
            slots = len(_GATES) * len(pieces) + _LEAD
            total = (D // 128) * NB * (NB + 1) // 2
            used = [0, 0]

            def pace():
                used[0] += 1
                while used[1] < total * used[0] // slots:
                    next(work)
                    used[1] += 1

            for _ in range(_LEAD):
                pace()
            for t, m in pieces:
                w = pltpu.bitcast(wk_v[g, :, t * 128:(t + 1) * 128], BF16)
                y = _dot(xa[m:m + _MB, :], w)
                for n, r in enumerate(_GATES):
                    xf[g, m // 2 + 8 * n:m // 2 + 8 * n + 8, ahead_lanes(1, t)] = y[r:r + 8]
                    pace()
                xf[g, m // 2:(m + _MB) // 2, ahead_lanes(1, t)] = pack_segments(y)
            for _ in work:
                pass
            transpose(2, g)
            return carry

        jax.lax.fori_loop(0, NP, products, 0)
        pltpu.make_async_copy(wo_hbm, wo_v, wo_sem).wait()

        skip = ssmd_ref[...].astype(F32).reshape(1, D)
        gw = gw_ref[...].astype(F32).reshape(1, D)
        h_v[0:M, :] = mem0_ref[...].astype(F32)

        row = jax.lax.broadcasted_iota(jnp.int32, (L, 2 * KR), 0)
        lane = jax.lax.broadcasted_iota(jnp.int32, (L, 2 * KR), 1)
        in_a = lane < KR
        col = jnp.where(in_a, lane, lane - KR)
        valid = col < L
        valid_a = valid & in_a
        valid_b = valid & (lane >= KR)
        allowed = (row < M) | (row >= col)
        dim_a = jax.lax.broadcasted_iota(jnp.int32, (L, PW), 1) < DH
        zpad = jnp.zeros((KR - L, PW), F32)

        def block_diag(t):
            a = jnp.where(dim_a, t, 0.0)
            b = jnp.where(dim_a, 0.0, t)
            return jnp.concatenate([a, zpad, b, zpad], axis=0).astype(BF16)

        def softmax(s):
            s = jnp.where(allowed, s * scale, -1e9)
            ma = jnp.max(jnp.where(valid_a, s, -jnp.inf), axis=1, keepdims=True)
            mb = jnp.max(jnp.where(valid_b, s, -jnp.inf), axis=1, keepdims=True)
            e = jnp.where(valid, jnp.exp(s - jnp.where(in_a, ma, mb)), 0.0)
            la = jnp.sum(jnp.where(in_a, e, 0.0), axis=1, keepdims=True)
            lb = jnp.sum(jnp.where(in_a, 0.0, e), axis=1, keepdims=True)
            return e * (1.0 / jnp.where(in_a, la, lb))

        def step(blk, part):
            rows = pl.ds(pl.multiple_of(blk * _T + part * SEG, SEG), SEG)
            ahead = pl.ds(pl.multiple_of((blk * (SPB // 2) + part // 2) * _AHEAD, _AHEAD), _AHEAD)
            xq = x_v[rows, :].astype(F32)
            h_v[M:L, :] = xq
            h = h_v[...]
            q, k, v, p, o = {}, {}, {}, {}, {}
            acc = []

            def project(i, j):
                w = pltpu.bitcast(qkv_v[j][i], BF16)
                if j == 2:
                    return _dot(h, w)
                word = pltpu.bitcast(xf[i, ahead, D + j * PW:D + (j + 1) * PW], U32)
                tail = word & U32(0xFFFF0000) if part % 2 else word << U32(16)
                return jnp.concatenate(
                    [_dot(h[0:L - _AHEAD], w), pltpu.bitcast(tail, F32)], axis=0)

            def project_out(i):
                y = _dot(o.pop(i), wo_v[i * PW:(i + 1) * PW, :])
                acc[:] = [y if not acc else acc[0] + y]

            conv = _dot(inv_ref[part * SEG:(part + 1) * SEG, :], xf[blk, :, 0:D].astype(BF16))
            g = jax.nn.sigmoid(jnp.sum(xq * gw, axis=1, keepdims=True))
            b = (1.0 - g) * (xq * (conv + kv_v[rows, :].astype(F32) * skip))

            for i in range(NP):
                k[i] = block_diag(project(i, 1))
                q[i] = project(i, 0)
                v[i] = block_diag(project(i, 2))
                if i >= 1:
                    o[i - 1] = _dot(p.pop(i - 1), v.pop(i - 1))
                p[i] = softmax(_dot(q.pop(i), k.pop(i), _NT))
                if 2 <= i < NP + 1 - _HELD:
                    project_out(i - 2)
            for i in range(NP - 1 - _HELD, NP - 2):
                project_out(i)
            o[NP - 1] = _dot(p.pop(NP - 1), v.pop(NP - 1))
            project_out(NP - 2)
            project_out(NP - 1)

            y = acc[0]
            h_v[0:M, :] = y[0:M].astype(BF16).astype(F32)
            out_v[rows, :] = (g * y[M:L] + b).astype(out_v.dtype)
            pltpu.make_async_copy(out_v.at[rows], o_hbm.at[rows], out_sem).start()

        def block(blk, carry):
            x_copy(blk).wait()

            @pl.when(blk + 1 < NB)
            def _():
                x_copy(blk + 1).start()

            for part in range(SPB):
                step(blk, part)
            return carry

        jax.lax.fori_loop(0, NB, block, 0)
        pltpu.make_async_copy(out_v, o_hbm, out_sem).wait()

    fwd_np, inv_np = _dft_matrices()
    hbm = pl.BlockSpec(memory_space=pl.ANY)
    vmem = pl.BlockSpec(memory_space=pltpu.VMEM)

    def head_major(w):
        return jnp.transpose(w, (1, 2, 0)).reshape(H * DH, D)

    out = pl.pallas_call(
        kernel,
        out_shape=jax.ShapeDtypeStruct((S, D), A_x.dtype),
        in_specs=[hbm, hbm, vmem, hbm, hbm, hbm, hbm, hbm, hbm,
                  vmem, hbm, vmem, vmem, vmem, vmem],
        out_specs=hbm,
        scratch_shapes=[
            pltpu.VMEM((S, D), BF16),
            pltpu.VMEM((NP, D // 2, PW), U32),
            pltpu.VMEM((NP, D // 2, PW), U32),
            pltpu.VMEM((NP, D // 2, PW), U32),
            pltpu.VMEM((H * DH, D), BF16),
            pltpu.VMEM((L, D), F32),
            pltpu.VMEM((S, D), BF16),
            pltpu.VMEM((S, D), A_x.dtype),
            pltpu.VMEM((3, H * DH, D), BF16),
            pltpu.VMEM((S, D), BF16),
            pltpu.VMEM((S, D), BF16),
            pltpu.VMEM((D, S), BF16),
            pltpu.VMEM((_T + 8, D), F32),
            pltpu.VMEM((NB, 2 * _T, D + 2 * PW), F32),
            pltpu.VMEM((NB, 2 * _T, D), F32),
            pltpu.VMEM((2 * HALF + 8, D), F32),
            pltpu.VMEM((NSEG, _AHEAD, D), BF16),
            pltpu.SemaphoreType.DMA((3, _SLOTS)),
            pltpu.SemaphoreType.DMA((_SLOTS,)),
            pltpu.SemaphoreType.DMA(()),
            pltpu.SemaphoreType.DMA(()),
            pltpu.SemaphoreType.DMA(()),
            pltpu.SemaphoreType.DMA(()),
        ],
        compiler_params=pltpu.CompilerParams(vmem_limit_bytes=124 * 1024 * 1024),
    )(
        A_x.reshape(S, D), A_x.reshape(NSEG, SEG, D), A_mem0.reshape(M, D),
        head_major(A_Wq), head_major(A_Wk), head_major(A_Wv), A_Wo.reshape(H * DH, D),
        B_k.reshape(S, D), B_v.reshape(S, D),
        B_shift_k.T, B_ssm_k, B_ssm_D, gate_w,
        jnp.asarray(fwd_np.astype(BF16)), jnp.asarray(inv_np),
    )
    return out.reshape(1, S, D)
```

```python
import numpy as np

import jax
import jax.numpy as jnp
import jax.experimental.pallas as pl
import jax.experimental.pallas.tpu as pltpu

F32 = jnp.float32
BF16 = jnp.bfloat16
U32 = jnp.uint32
_NN = (((1,), (0,)), ((), ()))
_NT = (((1,), (1,)), ((), ()))
_T = 128
_AHEAD = 8
_DIST = 2
_SLOTS = 4
_GROUP = 4
_MB, _GATES, _LEAD = 64, (0, 32), 6
_HELD = 4


def _dot(a, b, dims=_NN):
    return jax.lax.dot_general(a, b, dims, preferred_element_type=F32)


def _dft_matrices():
    f = np.arange(_T, dtype=np.float64)[:, None]
    n = np.arange(_T, dtype=np.float64)[None, :]
    theta = np.pi * (2.0 * f + 1.0) * n / (2.0 * _T)
    fwd = np.concatenate([np.cos(theta), -np.sin(theta)], axis=0)
    inv = np.concatenate([np.cos(theta).T, -np.sin(theta).T], axis=1) / _T
    return fwd.astype(np.float32), inv.astype(np.float32)


@jax.jit(static_argnames=("A_seg_len",))
def pallas_gated_mix__memory_aug_recurrent_mem_tr__ssm_conv_h3__prompt_kernel(
    A_x: jax.Array,
    A_mem0: jax.Array,
    A_Wq: jax.Array,
    A_Wk: jax.Array,
    A_Wv: jax.Array,
    A_Wo: jax.Array,
    A_seg_len: int,
    B_q: jax.Array,
    B_k: jax.Array,
    B_v: jax.Array,
    B_shift_k: jax.Array,
    B_ssm_k: jax.Array,
    B_ssm_D: jax.Array,
    gate_w: jax.Array,
):
    del B_q
    _, S, D = A_x.shape
    _, H, DH = A_Wq.shape
    M = A_mem0.shape[1]
    SEG = int(A_seg_len)
    KS = B_shift_k.shape[1]
    L = M + SEG
    NSEG = S // SEG
    NP = H // 2
    PW = 2 * DH
    NB = S // _T
    SPB = _T // SEG
    HALF = NSEG // 2 * _AHEAD
    scale = DH ** -0.5
    assert A_x.shape[0] == 1 and S % _T == 0 and _T % (2 * SEG) == 0 and H % 2 == 0
    assert PW % 128 == 0 and D % 128 == 0 and M % 8 == 0 and SEG % 16 == 0
    assert 2 * L <= 128 and KS <= 8 and NP == NB == _T // 8 and HALF == 2 * _T

    def kernel(x_hbm, xs_hbm, mem0_ref, wq_hbm, wk_hbm, wv_hbm, wo_hbm, bk_hbm, bv_hbm,
               shift_ref, ssmk_hbm, ssmd_ref, gw_ref, fwd_ref, inv_ref,
               o_hbm,
               x_v, wq_v, wk_v, wv_v, wo_v, h_v, kv_v, out_v,
               stage, bk_v, bv_v, ssmk_v, kpad, xf, kf, xa, xs_v,
               w_sems, b_sems, xs_sem, wo_sem, x_sem, out_sem):
        qkv_v = (wq_v, wk_v, wv_v)

        def pair_rows(p):
            return pl.ds(pl.multiple_of(p * PW, PW), PW)

        def block_rows(a):
            return pl.ds(pl.multiple_of(a * _T, _T), _T)

        def w_copy(j, p):
            src = (wq_hbm, wk_hbm, wv_hbm)[j]
            return pltpu.make_async_copy(
                src.at[pair_rows(p)], stage.at[j, pair_rows(p)], w_sems.at[j, p % _SLOTS])

        def wo_copy(p):
            return pltpu.make_async_copy(wo_hbm.at[pair_rows(p)], wo_v.at[pair_rows(p)], wo_sem)

        def b_copies(a):
            blk, sem = block_rows(a), b_sems.at[a % _SLOTS]
            return (pltpu.make_async_copy(ssmk_hbm.at[:, blk], ssmk_v.at[:, blk], sem),
                    pltpu.make_async_copy(bk_hbm.at[blk], bk_v.at[blk], sem),
                    pltpu.make_async_copy(bv_hbm.at[blk], bv_v.at[blk], sem))

        def x_copy(a):
            return pltpu.make_async_copy(x_hbm.at[block_rows(a)], x_v.at[block_rows(a)], x_sem)

        def start_first_phase_copies(a):
            for c in b_copies(a):
                c.start()
            w_copy(0, a).start()
            w_copy(1, a).start()

        def transpose(j, p):
            qkv_v[j][p] = pltpu.bitcast(stage[j, pair_rows(p), :].T, U32)

        def ahead_lanes(j, t):
            return slice(D + j * PW + t * 128, D + j * PW + (t + 1) * 128)

        def pack_segments(y):
            return pltpu.bitcast(y.astype(BF16), F32)

        xs_copy = pltpu.make_async_copy(xs_hbm.at[:, SEG - _AHEAD:SEG, :], xs_v, xs_sem)
        xs_copy.start()
        start_first_phase_copies(0)
        xs_copy.wait()
        for a in range(1, _DIST):
            start_first_phase_copies(a)
        for s in range(0, NSEG, 2):
            even, odd = (pltpu.bitcast(xs_v[s + i].astype(F32), U32) for i in range(2))
            xa[s * _AHEAD:(s + 2) * _AHEAD, :] = pltpu.bitcast((even >> U32(16)) | odd, BF16).astype(F32)
        fwd = fwd_ref[...]
        taps = shift_ref[...].astype(F32)
        kpad[0:8, :] = jnp.zeros((8, D), F32)

        def spectra(a, carry):
            for c in b_copies(a):
                c.wait()
            w_copy(0, a).wait()
            w_copy(1, a).wait()

            @pl.when(a + _DIST < NB)
            def _():
                start_first_phase_copies(a + _DIST)

            @pl.when(a + _DIST >= NB)
            def _():
                w_copy(2, a + _DIST - NB).start()
                wo_copy(a + _DIST - NB).start()

            blk = block_rows(a)
            kf[a] = _dot(fwd, ssmk_v[:, blk], _NT)
            kpad[8:8 + _T, :] = bk_v[blk, :].astype(F32)
            ksh = kpad[8:8 + _T, :] * taps[0:1]
            for j in range(1, KS):
                ksh = ksh + kpad[8 - j:8 - j + _T, :] * taps[j:j + 1]
            kpad[0:8, :] = kpad[_T:_T + 8, :]
            kv = (ksh * bv_v[blk, :].astype(F32)).astype(BF16)
            kv_v[blk, :] = kv
            for t in range(PW // 128):
                w = stage[0, pl.ds(pl.multiple_of(a * PW + t * 128, 128), 128), :]
                for m in (0, HALF):
                    xf[a, m // 2:(m + HALF) // 2, ahead_lanes(0, t)] = pack_segments(
                        _dot(xa[m:m + HALF, :], w, _NT))
                if t == 0:
                    xf[a, :, 0:D] = _dot(fwd, kv)
                if t == 1:
                    transpose(1, a)
                    spare = pl.ds(pl.multiple_of(2 * HALF + 8 * (a >> 20), 8), 8)
                    xa[spare, 0:128] = pltpu.bitcast(wk_v[a, D // 2 - 8:D // 2, PW - 128:PW], F32)
            transpose(0, a)
            return carry

        jax.lax.fori_loop(0, NB, spectra, 0)

        sub = jax.lax.broadcasted_iota(jnp.int32, (8, 128), 0)
        sign = (1 - 2 * (sub & 1)).astype(F32)

        def block_products(g):
            re = pl.ds(pl.multiple_of(g * 8, 8), 8)
            im = pl.ds(pl.multiple_of(_T + g * 8, 8), 8)
            for t in range(D // 128):
                ln = slice(t * 128, (t + 1) * 128)
                above = None
                for top in range(NB - 1, -1, -_GROUP):
                    z = {}
                    for a in range(top + 1):
                        xr, xi = xf[a, re, ln], xf[a, im, ln]
                        for c in range(top, max(top - _GROUP, a - 1), -1):
                            kr, ki = kf[c - a, re, ln], kf[c - a, im, ln]
                            tr, ti = xr * kr - xi * ki, xr * ki + xi * kr
                            z[c] = (tr, ti) if a == 0 else (z[c][0] + tr, z[c][1] + ti)
                            yield
                    for c in range(top, top - _GROUP, -1):
                        if above is not None:
                            xf[c + 1, re, ln] = above[0] - sign * z[c][1]
                            xf[c + 1, im, ln] = above[1] + sign * z[c][0]
                        above = z[c]
                xf[0, re, ln], xf[0, im, ln] = above

        def products(g, carry):
            w_copy(2, g).wait()

            @pl.when(g + _DIST < NP)
            def _():
                w_copy(2, g + _DIST).start()
                wo_copy(g + _DIST).start()

            @pl.when(g + _DIST == NP)
            def _():
                x_copy(0).start()

            work = block_products(g)
            pieces = [(t, m) for t in range(PW // 128) for m in range(0, 2 * HALF, _MB)]
            slots = len(_GATES) * len(pieces) + _LEAD
            total = (D // 128) * NB * (NB + 1) // 2
            used = [0, 0]

            def pace():
                used[0] += 1
                while used[1] < total * used[0] // slots:
                    next(work)
                    used[1] += 1

            for _ in range(_LEAD):
                pace()
            for t, m in pieces:
                w = pltpu.bitcast(wk_v[g, :, t * 128:(t + 1) * 128], BF16)
                y = _dot(xa[m:m + _MB, :], w)
                for n, r in enumerate(_GATES):
                    xf[g, m // 2 + 8 * n:m // 2 + 8 * n + 8, ahead_lanes(1, t)] = y[r:r + 8]
                    pace()
                xf[g, m // 2:(m + _MB) // 2, ahead_lanes(1, t)] = pack_segments(y)
            for _ in work:
                pass
            transpose(2, g)
            return carry

        jax.lax.fori_loop(0, NP, products, 0)
        pltpu.make_async_copy(wo_hbm, wo_v, wo_sem).wait()

        skip = ssmd_ref[...].astype(F32).reshape(1, D)
        gw = gw_ref[...].astype(F32).reshape(1, D)
        h_v[0:M, :] = mem0_ref[...].astype(F32)

        row = jax.lax.broadcasted_iota(jnp.int32, (L, 2 * L), 0)
        lane = jax.lax.broadcasted_iota(jnp.int32, (L, 2 * L), 1)
        in_a = lane < L
        allowed = (row < M) | (row >= jnp.where(in_a, lane, lane - L))
        dim_a = jax.lax.broadcasted_iota(jnp.int32, (L, PW), 1) < DH

        def block_diag(t):
            return jnp.concatenate(
                [jnp.where(dim_a, t, 0.0), jnp.where(dim_a, 0.0, t)], axis=0).astype(BF16)

        def softmax(s):
            s = jnp.where(allowed, s * scale, -1e9)
            ma = jnp.max(jnp.where(in_a, s, -jnp.inf), axis=1, keepdims=True)
            mb = jnp.max(jnp.where(in_a, -jnp.inf, s), axis=1, keepdims=True)
            e = jnp.exp(s - jnp.where(in_a, ma, mb))
            la = jnp.sum(jnp.where(in_a, e, 0.0), axis=1, keepdims=True)
            lb = jnp.sum(jnp.where(in_a, 0.0, e), axis=1, keepdims=True)
            return e * (1.0 / jnp.where(in_a, la, lb))

        def step(blk, part):
            rows = pl.ds(pl.multiple_of(blk * _T + part * SEG, SEG), SEG)
            ahead = pl.ds(pl.multiple_of((blk * (SPB // 2) + part // 2) * _AHEAD, _AHEAD), _AHEAD)
            xq = x_v[rows, :].astype(F32)
            h_v[M:L, :] = xq
            h = h_v[...]
            q, k, v, p, o = {}, {}, {}, {}, {}
            acc = []

            def project(i, j):
                w = pltpu.bitcast(qkv_v[j][i], BF16)
                n = L if j == 2 else L - _AHEAD
                y = _dot(jnp.concatenate([h[M:n], h[0:M]], axis=0), w)
                y = jnp.concatenate([y[n - M:n], y[0:n - M]], axis=0)
                if j == 2:
                    return y
                word = pltpu.bitcast(xf[i, ahead, D + j * PW:D + (j + 1) * PW], U32)
                tail = word & U32(0xFFFF0000) if part % 2 else word << U32(16)
                return jnp.concatenate(
                    [y, pltpu.bitcast(tail, F32)], axis=0)

            def project_out(i):
                y = _dot(o.pop(i), wo_v[i * PW:(i + 1) * PW, :])
                acc[:] = [y if not acc else acc[0] + y]

            conv = _dot(inv_ref[part * SEG:(part + 1) * SEG, :], xf[blk, :, 0:D].astype(BF16))
            g = jax.nn.sigmoid(jnp.sum(xq * gw, axis=1, keepdims=True))
            b = (1.0 - g) * (xq * (conv + kv_v[rows, :].astype(F32) * skip))

            parked = xf.at[NB + (blk >> 20)]
            for i in range(NP):
                if i == NP // 2:
                    parked[0:SEG, 0:D] = b
                    parked[0:SEG, D:D + 128] = jnp.broadcast_to(g, (SEG, 128))
                k[i] = block_diag(project(i, 1))
                q[i] = project(i, 0)
                v[i] = block_diag(project(i, 2))
                if i >= 1:
                    o[i - 1] = _dot(p.pop(i - 1), v.pop(i - 1))
                p[i] = softmax(_dot(q.pop(i), k.pop(i), _NT))
                if 2 <= i < NP + 1 - _HELD:
                    project_out(i - 2)
            for i in range(NP - 1 - _HELD, NP - 2):
                project_out(i)
            o[NP - 1] = _dot(p.pop(NP - 1), v.pop(NP - 1))
            project_out(NP - 2)
            project_out(NP - 1)

            y = acc[0]
            h_v[0:M, :] = y[0:M].astype(BF16).astype(F32)
            g = jnp.concatenate([parked[0:SEG, D:D + 128]] * (D // 128), axis=1)
            out_v[rows, :] = (g * y[M:L] + parked[0:SEG, 0:D]).astype(out_v.dtype)

        def block(blk, carry):
            x_copy(blk).wait()

            @pl.when(blk + 1 < NB)
            def _():
                x_copy(blk + 1).start()

            for part in range(SPB):
                step(blk, part)
            rows = block_rows(blk)
            pltpu.make_async_copy(out_v.at[rows], o_hbm.at[rows], out_sem).start()
            return carry

        jax.lax.fori_loop(0, NB, block, 0)
        pltpu.make_async_copy(out_v, o_hbm, out_sem).wait()

    fwd_np, inv_np = _dft_matrices()
    hbm = pl.BlockSpec(memory_space=pl.ANY)
    vmem = pl.BlockSpec(memory_space=pltpu.VMEM)

    def head_major(w):
        return jnp.transpose(w, (1, 2, 0)).reshape(H * DH, D)

    out = pl.pallas_call(
        kernel,
        out_shape=jax.ShapeDtypeStruct((S, D), A_x.dtype),
        in_specs=[hbm, hbm, vmem, hbm, hbm, hbm, hbm, hbm, hbm,
                  vmem, hbm, vmem, vmem, vmem, vmem],
        out_specs=hbm,
        scratch_shapes=[
            pltpu.VMEM((S, D), BF16),
            pltpu.VMEM((NP, D // 2, PW), U32),
            pltpu.VMEM((NP, D // 2, PW), U32),
            pltpu.VMEM((NP, D // 2, PW), U32),
            pltpu.VMEM((H * DH, D), BF16),
            pltpu.VMEM((L, D), F32),
            pltpu.VMEM((S, D), BF16),
            pltpu.VMEM((S, D), A_x.dtype),
            pltpu.VMEM((3, H * DH, D), BF16),
            pltpu.VMEM((S, D), BF16),
            pltpu.VMEM((S, D), BF16),
            pltpu.VMEM((D, S), BF16),
            pltpu.VMEM((_T + 8, D), F32),
            pltpu.VMEM((NB + 1, 2 * _T, D + 2 * PW), F32),
            pltpu.VMEM((NB, 2 * _T, D), F32),
            pltpu.VMEM((2 * HALF + 8, D), F32),
            pltpu.VMEM((NSEG, _AHEAD, D), BF16),
            pltpu.SemaphoreType.DMA((3, _SLOTS)),
            pltpu.SemaphoreType.DMA((_SLOTS,)),
            pltpu.SemaphoreType.DMA(()),
            pltpu.SemaphoreType.DMA(()),
            pltpu.SemaphoreType.DMA(()),
            pltpu.SemaphoreType.DMA(()),
        ],
        compiler_params=pltpu.CompilerParams(vmem_limit_bytes=112 * 1024 * 1024),
    )(
        A_x.reshape(S, D), A_x.reshape(NSEG, SEG, D), A_mem0.reshape(M, D),
        head_major(A_Wq), head_major(A_Wk), head_major(A_Wv), A_Wo.reshape(H * DH, D),
        B_k.reshape(S, D), B_v.reshape(S, D),
        B_shift_k.T, B_ssm_k, B_ssm_D, gate_w,
        jnp.asarray(fwd_np.astype(BF16)), jnp.asarray(inv_np),
    )
    return out.reshape(1, S, D)
```

```python
import numpy as np

import jax
import jax.numpy as jnp
import jax.experimental.pallas as pl
import jax.experimental.pallas.tpu as pltpu

F32 = jnp.float32
BF16 = jnp.bfloat16
U32 = jnp.uint32
_NN = (((1,), (0,)), ((), ()))
_NT = (((1,), (1,)), ((), ()))
_T = 128
_AHEAD = 8
_DIST = 2
_SLOTS = 4
_GROUP = 4
_MB, _GATES, _LEAD = 64, (0, 24, 48), 10
_HELD = 4


def _dot(a, b, dims=_NN):
    return jax.lax.dot_general(a, b, dims, preferred_element_type=F32)


def _dft_matrices():
    f = np.arange(_T, dtype=np.float64)[None, :, None]
    n = np.arange(4 * _T, dtype=np.float64).reshape(4, 1, _T)
    theta = np.pi * (2.0 * f + 1.0) * n / (2.0 * _T)
    fwd = np.concatenate([np.cos(theta), -np.sin(theta)], axis=1)
    return fwd.astype(np.float32), (fwd.transpose(0, 2, 1) / _T).astype(np.float32)


@jax.jit(static_argnames=("A_seg_len",))
def pallas_gated_mix__memory_aug_recurrent_mem_tr__ssm_conv_h3__prompt_kernel(
    A_x: jax.Array,
    A_mem0: jax.Array,
    A_Wq: jax.Array,
    A_Wk: jax.Array,
    A_Wv: jax.Array,
    A_Wo: jax.Array,
    A_seg_len: int,
    B_q: jax.Array,
    B_k: jax.Array,
    B_v: jax.Array,
    B_shift_k: jax.Array,
    B_ssm_k: jax.Array,
    B_ssm_D: jax.Array,
    gate_w: jax.Array,
):
    del B_q
    _, S, D = A_x.shape
    _, H, DH = A_Wq.shape
    M = A_mem0.shape[1]
    SEG = int(A_seg_len)
    KS = B_shift_k.shape[1]
    L = M + SEG
    NSEG = S // SEG
    NP = H // 2
    PW = 2 * DH
    NB = S // _T
    SPB = _T // SEG
    HALF = NSEG // 2 * _AHEAD
    scale = DH ** -0.5
    assert A_x.shape[0] == 1 and S % _T == 0 and _T % (2 * SEG) == 0 and H % 2 == 0
    assert PW % 128 == 0 and D % 128 == 0 and M % 8 == 0 and SEG % 16 == 0
    assert 2 * L <= 128 and KS <= 8 and NP == NB == _T // 8 and HALF == 2 * _T

    def kernel(x_hbm, xs_hbm, mem0_ref, wq_hbm, wk_hbm, wv_hbm, wo_hbm, bk_hbm, bv_hbm,
               shift_ref, ssmk_hbm, ssmd_ref, gw_ref, fwd_hbm, inv_hbm,
               o_hbm,
               x_v, wq_v, wk_v, wv_v, wo_v, h_v, kv_v, out_v,
               stage, bk_v, bv_v, ssmk_v, kpad, xf, kf, xa, xs_v, fwd_ref, inv_ref,
               w_sems, b_sems, xs_sem, wo_sem, x_sem, out_sem):
        qkv_v = (wq_v, wk_v, wv_v)

        def pair_rows(p):
            return pl.ds(pl.multiple_of(p * PW, PW), PW)

        def block_rows(a):
            return pl.ds(pl.multiple_of(a * _T, _T), _T)

        def w_copy(j, p):
            src = (wq_hbm, wk_hbm, wv_hbm)[j]
            return pltpu.make_async_copy(
                src.at[pair_rows(p)], stage.at[j, pair_rows(p)], w_sems.at[j, p % _SLOTS])

        def wo_copy(p):
            return pltpu.make_async_copy(wo_hbm.at[pair_rows(p)], wo_v.at[pair_rows(p)], wo_sem)

        def b_copies(a):
            blk, sem = block_rows(a), b_sems.at[a % _SLOTS]
            return (pltpu.make_async_copy(ssmk_hbm.at[:, blk], ssmk_v.at[:, blk], sem),
                    pltpu.make_async_copy(bk_hbm.at[blk], bk_v.at[blk], sem),
                    pltpu.make_async_copy(bv_hbm.at[blk], bv_v.at[blk], sem))

        def x_copy(a):
            return pltpu.make_async_copy(x_hbm.at[block_rows(a)], x_v.at[block_rows(a)], x_sem)

        def start_first_phase_copies(a):
            for c in b_copies(a):
                c.start()
            w_copy(0, a).start()
            w_copy(1, a).start()

        def transpose(j, p):
            qkv_v[j][p] = pltpu.bitcast(stage[j, pair_rows(p), :].T, U32)

        def ahead_lanes(j, t):
            return slice(D + j * PW + t * 128, D + j * PW + (t + 1) * 128)

        def pack_segments(y):
            return pltpu.bitcast(y.astype(BF16), F32)

        xs_copy = pltpu.make_async_copy(xs_hbm.at[:, SEG - _AHEAD:SEG, :], xs_v, xs_sem)
        fwd_copy = pltpu.make_async_copy(fwd_hbm, fwd_ref, xs_sem)
        xs_copy.start()
        fwd_copy.start()
        start_first_phase_copies(0)
        xs_copy.wait()
        fwd_copy.wait()
        for a in range(1, _DIST):
            start_first_phase_copies(a)
        for s in range(0, NSEG, 2):
            even, odd = (pltpu.bitcast(xs_v[s + i].astype(F32), U32) for i in range(2))
            xa[s * _AHEAD:(s + 2) * _AHEAD, :] = pltpu.bitcast((even >> U32(16)) | odd, BF16).astype(F32)
        taps = shift_ref[...].astype(F32)
        kpad[0:8, :] = jnp.zeros((8, D), F32)

        def spectra(a, carry):
            for c in b_copies(a):
                c.wait()
            w_copy(0, a).wait()
            w_copy(1, a).wait()

            @pl.when(a + _DIST < NB)
            def _():
                start_first_phase_copies(a + _DIST)

            @pl.when(a + _DIST >= NB)
            def _():
                w_copy(2, a + _DIST - NB).start()
                wo_copy(a + _DIST - NB).start()

            blk = block_rows(a)
            fwd = fwd_ref[a % 4]
            kf[a] = _dot(fwd, ssmk_v[:, blk], _NT)
            kpad[8:8 + _T, :] = bk_v[blk, :].astype(F32)
            ksh = kpad[8:8 + _T, :] * taps[0:1]
            for j in range(1, KS):
                ksh = ksh + kpad[8 - j:8 - j + _T, :] * taps[j:j + 1]
            kpad[0:8, :] = kpad[_T:_T + 8, :]
            kv = (ksh * bv_v[blk, :].astype(F32)).astype(BF16)
            kv_v[blk, :] = kv
            for t in range(PW // 128):
                w = stage[0, pl.ds(pl.multiple_of(a * PW + t * 128, 128), 128), :]
                for m in (0, HALF):
                    xf[a, m // 2:(m + HALF) // 2, ahead_lanes(0, t)] = pack_segments(
                        _dot(xa[m:m + HALF, :], w, _NT))
                if t == 0:
                    xf[a, :, 0:D] = _dot(fwd, kv)
                if t == 1:
                    transpose(1, a)
                    spare = pl.ds(pl.multiple_of(2 * HALF + 8 * (a >> 20), 8), 8)
                    xa[spare, 0:128] = pltpu.bitcast(wk_v[a, D // 2 - 8:D // 2, PW - 128:PW], F32)
            transpose(0, a)
            return carry

        jax.lax.fori_loop(0, NB, spectra, 0)

        def block_products(g):
            re = pl.ds(pl.multiple_of(g * 8, 8), 8)
            im = pl.ds(pl.multiple_of(_T + g * 8, 8), 8)
            for t in range(D // 128):
                ln = slice(t * 128, (t + 1) * 128)
                above = None
                for top in range(NB - 1, -1, -_GROUP):
                    z = {}
                    for a in range(top + 1):
                        xr, xi = xf[a, re, ln], xf[a, im, ln]
                        for c in range(top, max(top - _GROUP, a - 1), -1):
                            kr, ki = kf[c - a, re, ln], kf[c - a, im, ln]
                            if a == 0:
                                z[c] = (xr * kr - xi * ki, xr * ki + xi * kr)
                            else:
                                z[c] = (z[c][0] + xr * kr - xi * ki, z[c][1] + xr * ki + xi * kr)
                            yield
                    for c in range(top, top - _GROUP, -1):
                        if above is not None:
                            xf[c + 1, re, ln] = above[0] + z[c][0]
                            xf[c + 1, im, ln] = above[1] + z[c][1]
                        above = z[c]
                xf[0, re, ln], xf[0, im, ln] = above

        def products(g, carry):
            w_copy(2, g).wait()

            @pl.when(g + _DIST < NP)
            def _():
                w_copy(2, g + _DIST).start()
                wo_copy(g + _DIST).start()

            @pl.when(g + _DIST == NP)
            def _():
                x_copy(0).start()

            work = block_products(g)
            pieces = [(t, m) for t in range(PW // 128) for m in range(0, 2 * HALF, _MB)]
            slots = len(_GATES) * len(pieces) + _LEAD
            total = (D // 128) * NB * (NB + 1) // 2
            used = [0, 0]

            def pace():
                used[0] += 1
                while used[1] < total * used[0] // slots:
                    next(work)
                    used[1] += 1

            for _ in range(_LEAD):
                pace()
            for t, m in pieces:
                w = pltpu.bitcast(wk_v[g, :, t * 128:(t + 1) * 128], BF16)
                y = _dot(xa[m:m + _MB, :], w)
                for n, r in enumerate(_GATES):
                    xf[g, m // 2 + 8 * n:m // 2 + 8 * n + 8, ahead_lanes(1, t)] = y[r:r + 8]
                    pace()
                xf[g, m // 2:(m + _MB) // 2, ahead_lanes(1, t)] = pack_segments(y)
            for _ in work:
                pass
            transpose(2, g)
            return carry

        inv_copy = pltpu.make_async_copy(inv_hbm, inv_ref, xs_sem)
        inv_copy.start()
        jax.lax.fori_loop(0, NP, products, 0)
        inv_copy.wait()
        pltpu.make_async_copy(wo_hbm, wo_v, wo_sem).wait()

        skip = ssmd_ref[...].astype(F32).reshape(1, D)
        gw = gw_ref[...].astype(F32).reshape(1, D)
        h_v[0:M, :] = mem0_ref[...].astype(F32)

        row = jax.lax.broadcasted_iota(jnp.int32, (L, 2 * L), 0)
        lane = jax.lax.broadcasted_iota(jnp.int32, (L, 2 * L), 1)
        in_a = lane < L
        allowed = (row < M) | (row >= jnp.where(in_a, lane, lane - L))
        dim_a = jax.lax.broadcasted_iota(jnp.int32, (L, PW), 1) < DH

        def block_diag(t):
            return jnp.concatenate(
                [jnp.where(dim_a, t, 0.0), jnp.where(dim_a, 0.0, t)], axis=0).astype(BF16)

        def softmax(s):
            s = jnp.where(allowed, s * scale, -1e9)
            ma = jnp.max(jnp.where(in_a, s, -jnp.inf), axis=1, keepdims=True)
            mb = jnp.max(jnp.where(in_a, -jnp.inf, s), axis=1, keepdims=True)
            e = jnp.exp(s - jnp.where(in_a, ma, mb))
            la = jnp.sum(jnp.where(in_a, e, 0.0), axis=1, keepdims=True)
            lb = jnp.sum(jnp.where(in_a, 0.0, e), axis=1, keepdims=True)
            return e * (1.0 / jnp.where(in_a, la, lb))

        def step(blk, part):
            rows = pl.ds(pl.multiple_of(blk * _T + part * SEG, SEG), SEG)
            ahead = pl.ds(pl.multiple_of((blk * (SPB // 2) + part // 2) * _AHEAD, _AHEAD), _AHEAD)
            xq = x_v[rows, :].astype(F32)
            h_v[M:L, :] = xq
            h = h_v[...]
            q, k, v, p, o = {}, {}, {}, {}, {}
            acc = []

            def project(i, j):
                w = pltpu.bitcast(qkv_v[j][i], BF16)
                n = L if j == 2 else L - _AHEAD
                y = _dot(jnp.concatenate([h[M:n], h[0:M]], axis=0), w)
                y = jnp.concatenate([y[n - M:n], y[0:n - M]], axis=0)
                if j == 2:
                    return y
                word = pltpu.bitcast(xf[i, ahead, D + j * PW:D + (j + 1) * PW], U32)
                tail = word & U32(0xFFFF0000) if part % 2 else word << U32(16)
                return jnp.concatenate([y, pltpu.bitcast(tail, F32)], axis=0)

            def project_out(i):
                y = _dot(o.pop(i), wo_v[i * PW:(i + 1) * PW, :])
                acc[:] = [y if not acc else acc[0] + y]

            conv = _dot(inv_ref[blk % 4, part * SEG:(part + 1) * SEG, :], xf[blk, :, 0:D].astype(BF16))
            g = jax.nn.sigmoid(jnp.sum(xq * gw, axis=1, keepdims=True))
            b = (1.0 - g) * (xq * (conv + kv_v[rows, :].astype(F32) * skip))

            parked = xf.at[NB + (blk >> 20)]
            for i in range(NP):
                if i == NP // 2:
                    parked[0:SEG, 0:D] = b
                    parked[0:SEG, D:D + 128] = jnp.broadcast_to(g, (SEG, 128))
                k[i] = block_diag(project(i, 1))
                q[i] = project(i, 0)
                v[i] = block_diag(project(i, 2))
                if i >= 1:
                    o[i - 1] = _dot(p.pop(i - 1), v.pop(i - 1))
                p[i] = softmax(_dot(q.pop(i), k.pop(i), _NT))
                if 2 <= i < NP + 1 - _HELD:
                    project_out(i - 2)
            for i in range(NP - 1 - _HELD, NP - 2):
                project_out(i)
            o[NP - 1] = _dot(p.pop(NP - 1), v.pop(NP - 1))
            project_out(NP - 2)
            project_out(NP - 1)

            y = acc[0]
            h_v[0:M, :] = y[0:M].astype(BF16).astype(F32)
            g = jnp.concatenate([parked[0:SEG, D:D + 128]] * (D // 128), axis=1)
            out_v[rows, :] = (g * y[M:L] + parked[0:SEG, 0:D]).astype(out_v.dtype)

        def block(blk, carry):
            x_copy(blk).wait()

            @pl.when(blk + 1 < NB)
            def _():
                x_copy(blk + 1).start()

            for part in range(SPB):
                step(blk, part)
            rows = block_rows(blk)
            pltpu.make_async_copy(out_v.at[rows], o_hbm.at[rows], out_sem).start()
            return carry

        jax.lax.fori_loop(0, NB, block, 0)
        pltpu.make_async_copy(out_v, o_hbm, out_sem).wait()

    fwd_np, inv_np = _dft_matrices()
    hbm = pl.BlockSpec(memory_space=pl.ANY)
    vmem = pl.BlockSpec(memory_space=pltpu.VMEM)

    def head_major(w):
        return jnp.transpose(w, (1, 2, 0)).reshape(H * DH, D)

    out = pl.pallas_call(
        kernel,
        out_shape=jax.ShapeDtypeStruct((S, D), A_x.dtype),
        in_specs=[hbm, hbm, vmem, hbm, hbm, hbm, hbm, hbm, hbm,
                  vmem, hbm, vmem, vmem, hbm, hbm],
        out_specs=hbm,
        scratch_shapes=[
            pltpu.VMEM((S, D), BF16),
            pltpu.VMEM((NP, D // 2, PW), U32),
            pltpu.VMEM((NP, D // 2, PW), U32),
            pltpu.VMEM((NP, D // 2, PW), U32),
            pltpu.VMEM((H * DH, D), BF16),
            pltpu.VMEM((L, D), F32),
            pltpu.VMEM((S, D), BF16),
            pltpu.VMEM((S, D), A_x.dtype),
            pltpu.VMEM((3, H * DH, D), BF16),
            pltpu.VMEM((S, D), BF16),
            pltpu.VMEM((S, D), BF16),
            pltpu.VMEM((D, S), BF16),
            pltpu.VMEM((_T + 8, D), F32),
            pltpu.VMEM((NB + 1, 2 * _T, D + 2 * PW), F32),
            pltpu.VMEM((NB, 2 * _T, D), F32),
            pltpu.VMEM((2 * HALF + 8, D), F32),
            pltpu.VMEM((NSEG, _AHEAD, D), BF16),
            pltpu.VMEM((4, 2 * _T, _T), BF16),
            pltpu.VMEM((4, _T, 2 * _T), F32),
            pltpu.SemaphoreType.DMA((3, _SLOTS)),
            pltpu.SemaphoreType.DMA((_SLOTS,)),
            pltpu.SemaphoreType.DMA(()),
            pltpu.SemaphoreType.DMA(()),
            pltpu.SemaphoreType.DMA(()),
            pltpu.SemaphoreType.DMA(()),
        ],
        compiler_params=pltpu.CompilerParams(vmem_limit_bytes=112 * 1024 * 1024),
    )(
        A_x.reshape(S, D), A_x.reshape(NSEG, SEG, D), A_mem0.reshape(M, D),
        head_major(A_Wq), head_major(A_Wk), head_major(A_Wv), A_Wo.reshape(H * DH, D),
        B_k.reshape(S, D), B_v.reshape(S, D),
        B_shift_k.T, B_ssm_k, B_ssm_D, gate_w,
        jnp.asarray(fwd_np.astype(BF16)), jnp.asarray(inv_np),
    )
    return out.reshape(1, S, D)
```
